```python
import jax
import jax.numpy as jnp

def _softmax(x, axis=-1):
    return jax.nn.softmax(x, axis=axis)
def _gelu(x):
    return jax.nn.gelu(x, approximate=True)
def _silu(x):
    return jax.nn.silu(x)
def _sigmoid(x):
    return jax.nn.sigmoid(x)
def _layernorm(x, axis=-1, eps=1e-5):
    m = jnp.mean(x, axis=axis, keepdims=True)
    v = jnp.var(x, axis=axis, keepdims=True)
    return (x - m) / jnp.sqrt(v + eps)
def _scatter_add(tgt, idx, src, axis=0):
    return tgt.at[idx].add(src)
def _segment_sum(src, seg, n):
    return jax.ops.segment_sum(src, seg, n)
class _Rng:
    def __init__(self, key):
        self._k = key
    def _next(self):
        self._k, sub = jax.random.split(self._k)
        return sub
    def normal(self, shape):
        return jax.random.normal(self._next(), shape, dtype=jnp.bfloat16)
    def randint(self, lo, hi, shape):
        return jax.random.randint(self._next(), shape, lo, hi, dtype=jnp.int32)
    def uniform(self, shape, lo=0.0, hi=1.0):
        return jax.random.uniform(self._next(), shape, jnp.bfloat16, lo, hi)
    def permutation(self, n):
        return jax.random.permutation(self._next(), n)


kernel_name = 'standalone__modern_conv_block_convnext_v2__vision'

def setup_inputs():
    _rng = _Rng(jax.random.key(int.from_bytes(__import__("os").urandom(4), "little")))
    _w = (lambda a: (lambda t: t.astype(jnp.bfloat16) if jnp.issubdtype(t.dtype, jnp.floating) else t)(jnp.asarray(a)))
    H = W = 512
    C = 96
    K = 3
    return {
        "x": _w((lambda *s: _rng.normal(s) * 0.05)(1, H, W, C)),
        "dw": _w((lambda *s: _rng.normal(s) * 0.05)(K, K, C)),
        "w1": _w((lambda *s: _rng.normal(s) * 0.05)(C, 4 * C)),
        "w2": _w((lambda *s: _rng.normal(s) * 0.05)(4 * C, C)),
        "grn_gamma": _w((lambda *s: _rng.normal(s) * 0.05)(4 * C)),
        "grn_beta": _w((lambda *s: _rng.normal(s) * 0.05)(4 * C)),
    }

def reference(x, dw, w1, w2, grn_gamma, grn_beta):
    B, H, W, C = x.shape
    K = dw.shape[0]
    pad = K // 2
    xp = jnp.pad(x, ((0,0),(pad,pad),(pad,pad),(0,0)))
    out = jnp.zeros_like(x)
    for i in range(K):
        for j in range(K):
            out = out + xp[:, i:i+H, j:j+W, :] * dw[i, j][None, None, None, :]
    h = _layernorm(out, axis=-1)
    h = jnp.einsum('bhwc,ce->bhwe', h, w1)
    h = _gelu(h)
    gx = jnp.sqrt((h * h).sum(axis=(1, 2), keepdims=True) + 1e-6)
    nx = gx / (gx.mean(axis=-1, keepdims=True) + 1e-6)
    h = grn_gamma * (h * nx) + grn_beta + h
    h = jnp.einsum('bhwe,ec->bhwc', h, w2)
    return x + h
```

```python
import functools
import math

import jax
import jax.numpy as jnp
import jax.experimental.pallas as pl
import jax.experimental.pallas.tpu as pltpu

_K0 = math.sqrt(2.0 / math.pi)
_K1 = 0.044715 * _K0
_ALPHA = _K1 ** (1.0 / 3.0)
_KP = _K0 / _ALPHA
_GS = 2.0 * _ALPHA


def _kernel(x_ref, xt_ref, xb_ref, dw_ref, w1_ref, w2t_ref, gam_ref, bet_ref,
            o_ref,
            g_s, acc_s, w1t_s, w2s_s, dwb_s, bias_s,
            *, TH, NR, NB, C, E, W):
    phase = pl.program_id(0)
    blk = pl.program_id(1)
    NRES = TH - NR
    f32 = jnp.float32
    bf16 = jnp.bfloat16

    @pl.when(jnp.logical_and(phase == 0, blk == 0))
    def _init():
        acc_s[...] = jnp.zeros(acc_s.shape, f32)
        w1t_s[...] = jnp.transpose(w1_ref[...].astype(f32)).astype(bf16)
        rows = jax.lax.broadcasted_iota(jnp.int32, (C, C), 0)
        cols = jax.lax.broadcasted_iota(jnp.int32, (C, C), 1)
        eye = rows == cols
        for i in range(3):
            for j in range(3):
                d = dw_ref[i, j:j + 1, :].astype(f32)
                col = jnp.sum(jnp.where(eye, d, 0.0), axis=1, keepdims=True)
                dwb_s[i * 3 + j] = jnp.broadcast_to(col, (C, 128))

    lane = jax.lax.broadcasted_iota(jnp.int32, (C, W), 1)

    def get_row(r):
        if r == -1:
            v = xt_ref[0].astype(f32)
            return jnp.where(blk > 0, v, 0.0)
        if r == TH:
            v = xb_ref[0].astype(f32)
            return jnp.where(blk < NB - 1, v, 0.0)
        return x_ref[r].astype(f32)

    def wt(i, j):
        w = dwb_s[i * 3 + j]
        return jnp.concatenate([w] * (W // 128), axis=1)

    def conv_ln(rows3):
        t = [rows3[0] * wt(0, j) + rows3[1] * wt(1, j) + rows3[2] * wt(2, j) for j in range(3)]
        left = pltpu.roll(jnp.where(lane == W - 1, 0.0, t[0]), 1, 1)
        right = pltpu.roll(jnp.where(lane == 0, 0.0, t[2]), W - 1, 1)
        o = t[1] + left + right
        m = jnp.sum(o, axis=0, keepdims=True) * (1.0 / C)
        d = o - m
        v = jnp.sum(d * d, axis=0, keepdims=True) * (1.0 / C)
        r = jax.lax.rsqrt(v + 1e-5) * _ALPHA
        return (d * r).astype(bf16)

    def gelu_stage(y):
        h = jnp.dot(w1t_s[...], y, preferred_element_type=f32)
        u = h * (h * h + _KP)
        return h * (1.0 + jnp.tanh(u))

    @pl.when(phase == 0)
    def _p1():
        for r in range(TH):
            y = conv_ln([get_row(r - 1), get_row(r), get_row(r + 1)])
            g = gelu_stage(y)
            g2 = g * g
            a = acc_s[...]
            for k in range(W // 128):
                a = a + g2[:, k * 128:(k + 1) * 128]
            acc_s[...] = a
            if r >= NR:
                g_s[blk * NRES + (r - NR)] = g.astype(bf16)

    @pl.when(jnp.logical_and(phase == 1, blk == 0))
    def _fin():
        ssq = jnp.sum(jnp.transpose(acc_s[...]), axis=0, keepdims=True)
        gx = jnp.sqrt(ssq * (1.0 / (_GS * _GS)) + 1e-6)
        nx = gx / (jnp.sum(gx, axis=1, keepdims=True) * (1.0 / E) + 1e-6)
        s = (gam_ref[...].astype(f32) * nx + 1.0) * (1.0 / _GS)
        w2 = w2t_ref[...].astype(f32)
        w2s_s[...] = (w2 * s).astype(bf16)
        b = jnp.sum(w2 * bet_ref[...].astype(f32), axis=1, keepdims=True)
        bias_s[...] = jnp.broadcast_to(b, (C, 128))

    @pl.when(phase == 1)
    def _p2():
        bias = jnp.concatenate([bias_s[...]] * (W // 128), axis=1)
        for r in range(TH):
            if r < NR:
                y = conv_ln([get_row(r - 1), get_row(r), get_row(r + 1)])
                g = gelu_stage(y).astype(bf16)
            else:
                g = g_s[blk * NRES + (r - NR)]
            p = jnp.dot(w2s_s[...], g, preferred_element_type=f32)
            o_ref[r] = (x_ref[r].astype(f32) + (p + bias)).astype(bf16)


@jax.jit
def pallas_standalone__modern_conv_block_convnext_v2__vision_kernel(
    x: jax.Array,
    dw: jax.Array,
    w1: jax.Array,
    w2: jax.Array,
    grn_gamma: jax.Array,
    grn_beta: jax.Array,
):
    B, H, W, C = x.shape
    E = w1.shape[1]
    assert B == 1
    TH = 8
    NR = 4
    NB = H // TH
    xt = jnp.transpose(x[0], (0, 2, 1))
    w2t = jnp.transpose(w2)
    gam = grn_gamma.reshape(1, E)
    bet = grn_beta.reshape(1, E)

    kern = functools.partial(_kernel, TH=TH, NR=NR, NB=NB, C=C, E=E, W=W)
    out = pl.pallas_call(
        kern,
        grid=(2, NB),
        in_specs=[
            pl.BlockSpec((TH, C, W), lambda p, i: (i, 0, 0)),
            pl.BlockSpec((1, C, W), lambda p, i: (jnp.maximum(i * TH - 1, 0), 0, 0)),
            pl.BlockSpec((1, C, W), lambda p, i: (jnp.minimum(i * TH + TH, H - 1), 0, 0)),
            pl.BlockSpec((3, 3, C), lambda p, i: (0, 0, 0)),
            pl.BlockSpec((C, E), lambda p, i: (0, 0)),
            pl.BlockSpec((C, E), lambda p, i: (0, 0)),
            pl.BlockSpec((1, E), lambda p, i: (0, 0)),
            pl.BlockSpec((1, E), lambda p, i: (0, 0)),
        ],
        out_specs=pl.BlockSpec((TH, C, W), lambda p, i: (i * p, 0, 0)),
        out_shape=jax.ShapeDtypeStruct((H, C, W), jnp.bfloat16),
        scratch_shapes=[
            pltpu.VMEM((NB * (TH - NR), E, W), jnp.bfloat16),
            pltpu.VMEM((E, 128), jnp.float32),
            pltpu.VMEM((E, C), jnp.bfloat16),
            pltpu.VMEM((C, E), jnp.bfloat16),
            pltpu.VMEM((9, C, 128), jnp.float32),
            pltpu.VMEM((C, 128), jnp.float32),
        ],
        compiler_params=pltpu.CompilerParams(
            dimension_semantics=("arbitrary", "arbitrary"),
            vmem_limit_bytes=120 * 1024 * 1024,
        ),
        name="convnext_block",
    )(xt, xt, xt, dw, w1, w2t, gam, bet)
    return jnp.transpose(out, (0, 2, 1))[None]
```

```python
import functools
import math

import jax
import jax.numpy as jnp
import jax.experimental.pallas as pl
import jax.experimental.pallas.tpu as pltpu

_K0 = math.sqrt(2.0 / math.pi)
_K1 = 0.044715 * _K0
_ALPHA = _K1 ** (1.0 / 3.0)
_KP = _K0 / _ALPHA
_GS = 2.0 * _ALPHA

f32 = jnp.float32
bf16 = jnp.bfloat16
u32 = jnp.uint32

NP = 8
NR = 4
TH = 8
RC = (1, 2, 3)
CH = 128
P2 = 'r0002,r0002,r0002,r0002,x222,r0002,y2,a,z,b,c'
NODMA2 = 0
SLOTMODE = 0
CSPLIT = 0
GLESS = 0
N1 = 256 // NP
N2 = 64
DIST = [8,8,8,8,8,8]
DIST0 = [0,8,10,10,10,10]
DISTL = [10,10,10,10,8,0]

_TAPS = [(0, 0), (0, 1), (0, 2), (1, 0), (1, 2), (2, 0), (2, 1), (2, 2)]


def _tree_sum(vs):
    vs = list(vs)
    while len(vs) > 1:
        nxt = [vs[i] + vs[i + 1] for i in range(0, len(vs) - 1, 2)]
        if len(vs) % 2:
            nxt.append(vs[-1])
        vs = nxt
    return vs[0]


def _sub_allreduce(s):
    s = s + pltpu.roll(s, 4, 0)
    s = s + pltpu.roll(s, 2, 0)
    s = s + pltpu.roll(s, 1, 0)
    return s


def _layernorm_tile(o, C, scale):
    m = _sub_allreduce(_tree_sum(o)) * (1.0 / C)
    d = [t - m for t in o]
    v = _sub_allreduce(_tree_sum([t * t for t in d]))
    r = jax.lax.rsqrt(v + C * 1e-5) * scale
    return jnp.concatenate([t * r for t in d], axis=0).astype(bf16)


def _gelu2(h):
    return h * (1.0 + jnp.tanh(h * (h * h + _KP)))


def _kernel(xp_hbm, x_hbm, par_ref, w1_ref, w2t_ref,
            o_hbm,
            g_s, acc_s, w1t_s, w2s_s, dwc_s, bias_s, l1_s, l2_s, lr_s, y_s,
            sem_c, sem_x, sem_o,
            *, H, C, E, W):
    NB1 = H // (2 * NP)
    NB = H // TH
    NG = C // 8
    NT = W // 128
    NS = NG * NT // 2
    NCH = E // CH
    res_rows = [r for r in range(TH) if r not in RC]
    NRES = len(res_rows)
    ln_scale = _ALPHA * math.sqrt(C)

    g_b = g_s.bitcast(bf16)
    y_b = y_s.bitcast(bf16)
    lane = jax.lax.broadcasted_iota(jnp.int32, (8, 128), 1)
    sub = jax.lax.broadcasted_iota(jnp.int32, (8, 128), 0)
    zero_u = jnp.zeros((8, 128), u32)

    def mm1_raw(y, c):
        lhs = pltpu.bitcast(w1t_s[c * CH // 2:(c + 1) * CH // 2, :], bf16)
        return jnp.dot(lhs, y, preferred_element_type=f32)

    def setup(dwb_s):
        acc_s[...] = jnp.zeros(acc_s.shape, f32)
        w1t_s[...] = pltpu.bitcast(jnp.transpose(w1_ref[...].astype(f32)).astype(bf16), u32)
        rows = jax.lax.broadcasted_iota(jnp.int32, (C, C), 0)
        cols = jax.lax.broadcasted_iota(jnp.int32, (C, C), 1)
        eye = rows == cols
        par = par_ref[...].astype(f32)
        for i in range(3):
            for j in range(3):
                d = par[2 + i * 3 + j:3 + i * 3 + j, 0:C]
                col = jnp.sum(jnp.where(eye, d, 0.0), axis=1, keepdims=True)
                dwb_s[i * 3 + j] = jnp.broadcast_to(col, (C, 128))
        r16 = jax.lax.broadcasted_iota(jnp.int32, (16, 128), 0)
        c16 = jax.lax.broadcasted_iota(jnp.int32, (16, 128), 1)
        kv = c16 // 16
        kb = c16 % 16
        k_row = 2 * (kv // 3) + kb // 8 - r16 // 8
        k_j = kv % 3
        for cg in range(NG):
            l1 = jnp.zeros((16, 128), f32)
            l2 = jnp.zeros((16, 128), f32)
            for i in range(3):
                for j in range(3):
                    w8 = dwb_s[i * 3 + j, cg * 8:cg * 8 + 8, :]
                    w16 = jnp.concatenate([w8, w8], axis=0)
                    hit = (kb % 8 == r16 % 8) & (k_row == i) & (k_j == j) & (kv < 6)
                    l1 = jnp.where(hit, w16, l1)
                    if (i, j) in _TAPS:
                        l2 = jnp.where(c16 == r16 + 16 * _TAPS.index((i, j)), w16, l2)
            l1_s[cg] = pltpu.bitcast(l1.astype(bf16), u32)
            l2_s[cg] = pltpu.bitcast(l2.astype(bf16), u32)
        dwc_s[...] = dwb_s[4]
        lr_s[...] = jnp.zeros(lr_s.shape, u32)
        y_s[...] = jnp.zeros(y_s.shape, u32)

    def gelu_acc(h, c, gidx):
        g = _gelu2(h)
        g2 = g * g
        acc_s[c * CH:(c + 1) * CH, :] += _tree_sum(
            [g2[:, k * 128:(k + 1) * 128] for k in range(NT)])
        if gidx is not None:
            g_b.at[gidx][c * CH:(c + 1) * CH, :] = g.astype(bf16)

    def gindex(blk, r):
        if r % TH not in res_rows:
            return None
        b = blk * (2 * NP // TH) + r // TH
        if r < 0:
            b = jnp.maximum(b, 0)
        return b * NRES + res_rows.index(r % TH)

    def pass1(cbuf, zb_s, cl_s, dwb_s):
        cu = cbuf.bitcast(u32)

        def c_copies(blk, slot):
            return [
                pltpu.make_async_copy(xp_hbm.at[pl.ds(blk * NP - 1, NP), 1],
                                      cbuf.at[slot, :, :, pl.ds(0, 8), :], sem_c.at[slot, 0]),
                pltpu.make_async_copy(xp_hbm.at[pl.ds(blk * NP, NP), 0],
                                      cbuf.at[slot, :, :, pl.ds(8, 8), :], sem_c.at[slot, 1]),
            ]

        def last_copy(slot):
            return pltpu.make_async_copy(xp_hbm.at[NB1 * NP - 1, 1],
                                         cbuf.at[slot, 0, :, pl.ds(0, 8), :], sem_c.at[slot, 0])

        pltpu.make_async_copy(xp_hbm.at[pl.ds(0, NP), 0],
                              cbuf.at[0, :, :, pl.ds(8, 8), :], sem_c.at[0, 1]).start()
        pltpu.make_async_copy(xp_hbm.at[pl.ds(0, NP - 1), 1],
                              cbuf.at[0, pl.ds(1, NP - 1), :, pl.ds(0, 8), :], sem_c.at[0, 0]).start()
        zb_s[...] = jnp.zeros(zb_s.shape, bf16)
        pltpu.make_async_copy(zb_s, cbuf.at[0, 0, :, pl.ds(0, 8), :], sem_c.at[0, 0]).start()
        setup(dwb_s)
        cl_s[...] = jnp.zeros(cl_s.shape, u32)

        def a1(slot, q):
            for cg in range(NG):
                t = [cu[slot, q, cg * NT + k] for k in range(NT)]
                for k in range(NT):
                    lo = (cg * NT + k) * 8
                    if q == NP - 1:
                        cl_s[lo:lo + 8, :] = t[k]
                    lsrc = t[k - 1] if k > 0 else zero_u
                    rsrc = t[k + 1] if k < NT - 1 else zero_u
                    lr_s[q % NR, 0, lo:lo + 8, :] = pltpu.roll(jnp.where(lane == 127, lsrc, t[k]), 1, 1)
                    lr_s[q % NR, 1, lo:lo + 8, :] = pltpu.roll(jnp.where(lane == 0, rsrc, t[k]), 127, 1)

        def conv_pair_dot(slot, j, cg, k):
            n = cg * NT + k
            parts = []
            for q in (j, j + 1):
                c = cu[slot, q, n] if q >= 0 else cl_s[8 * n:8 * n + 8, :]
                parts += [lr_s[q % NR, 0, 8 * n:8 * n + 8, :], c, lr_s[q % NR, 1, 8 * n:8 * n + 8, :]]
            wt = pltpu.bitcast(jnp.concatenate(parts, axis=0), bf16)
            lhs = pltpu.bitcast(l1_s[cg, :, 0:96], bf16)
            return jnp.dot(lhs, wt, preferred_element_type=f32)

        def b_and_c(slot, j, scale, yslot, gidx, dist):
            order = [(k, cg) for k in range(NT) for cg in range(NG)]
            o = {}
            pos = 0
            for n in range(2 * NCH):
                gelu_acc(mm1_raw(y_b[yslot, n // NCH], n % NCH), n % NCH, gidx[n // NCH])
                for (k, cg) in order[pos:pos + dist[n]]:
                    o[cg] = conv_pair_dot(slot, j, cg, k)
                    if cg == NG - 1:
                        for hh in range(2):
                            yt = _layernorm_tile([o[q][8 * hh:8 * hh + 8] for q in range(NG)], C, scale)
                            y_b.at[j % NR, hh][:, k * 128:(k + 1) * 128] = yt
                pos += dist[n]

        def body(i, carry):
            slot = i & 1
            for c in c_copies(i, slot):
                c.wait()

            @pl.when(i + 1 < NB1)
            def _():
                for c in c_copies(i + 1, 1 - slot):
                    c.start()

            @pl.when(i + 1 == NB1)
            def _():
                last_copy(1 - slot).start()

            for j in range(-1, NP - 1):
                scale = jnp.where(i > 0, ln_scale, 0.0) if j == -1 else ln_scale
                a1(slot, j + 1)
                jc = j - 2
                b_and_c(slot, j, scale, jc % NR, [gindex(i, 2 * jc), gindex(i, 2 * jc + 1)],
                        DIST0 if j == -1 else (DISTL if j == NP - 2 else DIST))
            return carry

        jax.lax.fori_loop(0, N1, body, 0)

        slot = NB1 % 2
        last_copy(slot).wait()
        cbuf[slot, 0, :, pl.ds(8, 8), :] = jnp.zeros((NG * NT, 8, 128), bf16)
        a1(slot, 0)
        b_and_c(slot, -1, ln_scale, (-3) % NR, [gindex(NB1, -6), gindex(NB1, -5)], DIST0)

    pl.run_scoped(
        pass1,
        pltpu.VMEM((2, NP, NG * NT, 16, 128), bf16),
        pltpu.VMEM((NG * NT, 8, 128), bf16),
        pltpu.VMEM((NG * NT * 8, 128), u32),
        pltpu.VMEM((9, C, 128), f32),
    )

    def pass2(xbuf, obuf, gt_s):
        xu = xbuf.bitcast(u32)
        gt_b = gt_s.bitcast(bf16)

        def x_copy(blk, slot):
            return pltpu.make_async_copy(x_hbm.at[pl.ds(blk * TH, TH)], xbuf.at[slot], sem_x.at[slot])

        def o_copy(blk, slot):
            return pltpu.make_async_copy(obuf.at[slot], o_hbm.at[pl.ds(blk * TH, TH)], sem_o.at[slot])

        x_copy(0, 0).start()
        x_copy(1, 1).start()

        for jc in (-2, -1):
            for n in range(2 * NCH):
                gelu_acc(mm1_raw(y_b[jc % NR, n // NCH], n % NCH), n % NCH,
                         gindex(NB1, 2 * jc + n // NCH))

        ssq = jnp.sum(jnp.transpose(acc_s[...]), axis=0, keepdims=True)
        gx = jnp.sqrt(ssq * (1.0 / (_GS * _GS)) + 1e-6)
        nx = gx / (jnp.sum(gx, axis=1, keepdims=True) * (1.0 / E) + 1e-6)
        par = par_ref[...].astype(f32)
        sc = (par[0:1, 0:E] * nx + 1.0) * (1.0 / _GS)
        w2 = w2t_ref[...].astype(f32)
        w2s_s[0:C // 2, :] = pltpu.bitcast((w2 * sc).astype(bf16), u32)
        b = jnp.sum(w2 * par[1:2, 0:E], axis=1, keepdims=True)
        bias_s[...] = jnp.broadcast_to(b, (C, 128))

        def xs_idx(r, v, s):
            n = 2 * (r - RC[0] + 1) + v
            return (n // 4, (n % 4) // 2, pl.ds((n % 2) * NS * 8 + 8 * s, 8), slice(None))

        def shift_rows(slot, rows):
            for s in [2 * cg + pp for pp in range(NT // 2) for cg in range(NG)]:
              for r in rows:
                a = xu[slot, r, 8 * s:8 * s + 8, :]
                bl = xu[slot, r, 8 * s - 4:8 * s + 4, :] if s > 0 else pltpu.roll(a, 4, 0)
                br = xu[slot, r, 8 * s + 4:8 * s + 12, :] if s < NS - 1 else pltpu.roll(a, 4, 0)
                if s % 2 == 0:
                    bl = jnp.where(sub < 4, zero_u, bl)
                else:
                    br = jnp.where(sub >= 4, zero_u, br)
                lr_s[xs_idx(r, 0, s)] = pltpu.roll(jnp.where(lane == 127, bl, a), 1, 1)
                lr_s[xs_idx(r, 1, s)] = pltpu.roll(jnp.where(lane == 0, br, a), 127, 1)

        def conv_dot(slot, r, s):
            cg = s // 2
            parts = []
            for (i, j) in _TAPS:
                rr = r + i - 1
                if j == 1:
                    parts.append(xu[slot, rr, 8 * s:8 * s + 8, :])
                else:
                    parts.append(lr_s[xs_idx(rr, j // 2, s)])
            wt = pltpu.bitcast(jnp.concatenate(parts, axis=0), bf16)
            lhs = pltpu.bitcast(l2_s[cg], bf16)
            p = jnp.dot(lhs, wt, preferred_element_type=f32)
            xc = pltpu.bitcast(xu[slot, r, 8 * s:8 * s + 8, :], bf16).astype(f32)
            w8 = dwc_s[cg * 8:cg * 8 + 8, :]
            return [p[0:8] + xc[0:8] * w8, p[8:16] + xc[8:16] * w8]

        def conv_ln_gen(slot, r, n):
            cnt = 0
            for pp in range(NT // 2):
                o = []
                for cg in range(NG):
                    o.append(conv_dot(slot, r, 2 * cg + pp))
                    cnt += 1
                    if cg == NG - 1:
                        for h in range(2):
                            k = 2 * pp + h
                            y_b.at[n // 2, n % 2][:, k * 128:(k + 1) * 128] = _layernorm_tile(
                                [o[q][h] for q in range(NG)], C, ln_scale)
                    if cnt % 4 == 0:
                        yield

        def stage_d(slot, oslot, r, g, gen, per):
            lhs = pltpu.bitcast(w2s_s[0:C // 2, :], bf16)
            p = []
            full = sum(per[:NT - 1]) == 0
            if full:
                pf = jnp.dot(lhs, g, preferred_element_type=f32)
            for k in range(NT):
                if full:
                    p.append(pf[:, k * 128:(k + 1) * 128])
                else:
                    p.append(jnp.dot(lhs, g[:, k * 128:(k + 1) * 128], preferred_element_type=f32))
                for _ in range(per[k]):
                    next(gen)
                if k % 2 == 1:
                    pp = k // 2
                    for cg in range(NG):
                        b8 = bias_s[cg * 8:cg * 8 + 8, :]
                        s = 2 * cg + pp
                        xr = pltpu.bitcast(xu[slot, r, 8 * s:8 * s + 8, :], bf16).astype(f32)
                        v = [xr[8 * h:8 * h + 8] + (p[2 * pp + h][cg * 8:cg * 8 + 8] + b8)
                             for h in range(2)]
                        obuf[oslot, r, 16 * s:16 * s + 16, :] = jnp.concatenate(v, axis=0).astype(bf16)

        def body(i, slot):
            oslot = i & 1
            if SLOTMODE == 1:
                slot = jax.lax.rem(i, 3)
            if SLOTMODE == 2:
                slot = i & 1
            if SLOTMODE == 3:
                slot = (i & 1) + 1
            if SLOTMODE == 5:
                slot = (i & 1) ^ 1
            if SLOTMODE == 6:
                slot = 2 - (i & 1)
            if SLOTMODE == 7:
                slot = (i >> 1) & 1
            if SLOTMODE == 4:
                slot = (i & 1) * 2
            if not NODMA2 & 1:
                x_copy(i, slot).wait()

            if not NODMA2 & 2:
                @pl.when(i >= 2)
                def _():
                    o_copy(i - 2, oslot).wait()

            if not NODMA2 & 1:
                @pl.when(i + 2 < NB)
                def _():
                    x_copy(i + 2, jnp.where(slot == 0, 2, slot - 1)).start()

            res = list(res_rows)

            def c_row(n, gen, per):
                if sum(per) == 0 and not CSPLIT:
                    lhs = pltpu.bitcast(w1t_s[...], bf16)
                    return [_gelu2(jnp.dot(lhs, y_b[n // 2, n % 2], preferred_element_type=f32))]
                out = []
                for c in range(NCH):
                    out.append(_gelu2(mm1_raw(y_b[n // 2, n % 2], c)))
                    for _ in range(per[c]):
                        next(gen)
                return out

            shift_rows(slot, range(RC[0] - 1, RC[0] + 2))
            for r in range(RC[0] + 2, RC[-1] + 2):
                shift_rows(slot, [r])
            gens = [conv_ln_gen(slot, r, n) for n, r in enumerate(RC)]

            def chain():
                for g_ in gens:
                    yield from g_
            ch = chain()
            for tok in P2.split(','):
                op = tok[0]
                per = [int(c) for c in tok[1:]] + [0] * 4
                if op == 'r':
                    r = res.pop(0)
                    stage_d(slot, oslot, r, g_b[i * NRES + res_rows.index(r)], ch, per)
                elif op in 'xyz':
                    n = 'xyz'.index(op)
                    gl = c_row(n, ch, per)
                    lo = 0
                    for gg in gl:
                        gt_b.at[n][lo:lo + gg.shape[0], :] = gg.astype(bf16)
                        lo += gg.shape[0]
                else:
                    n = 'abc'.index(op)
                    stage_d(slot, oslot, RC[n], gt_b[n], ch, per)
            assert not res and next(ch, 'done') == 'done'
            if not NODMA2 & 2:
                o_copy(i, oslot).start()
            return jnp.where(slot == 2, 0, slot + 1)

        jax.lax.fori_loop(0, N2, body, 0)
        if NODMA2 & 2:
            o_copy(0, 0).start()
            o_copy(1, 1).start()
        o_copy(N2 - 2, N2 % 2).wait()
        o_copy(N2 - 1, (N2 - 1) % 2).wait()
        if NODMA2 & 1:
            x_copy(0, 0).wait()
            x_copy(1, 1).wait()
        if N2 < NB:
            x_copy(N2, N2 % 3).wait()
        if N2 + 1 < NB:
            x_copy(N2 + 1, (N2 + 1) % 3).wait()

    pl.run_scoped(
        pass2,
        pltpu.VMEM((3, TH, NS * 16, 128), bf16),
        pltpu.VMEM((2, TH, NS * 16, 128), bf16),
        pltpu.VMEM((len(RC), E // 2, W), u32),
    )


@jax.jit
def pallas_standalone__modern_conv_block_convnext_v2__vision_kernel(
    x: jax.Array,
    dw: jax.Array,
    w1: jax.Array,
    w2: jax.Array,
    grn_gamma: jax.Array,
    grn_beta: jax.Array,
):
    B, H, W, C = x.shape
    E = w1.shape[1]
    assert B == 1
    NB = H // TH
    NG = C // 8
    NT = W // 128
    Q = NG * NT * 8
    x5 = jnp.transpose(x[0], (0, 2, 1)).reshape(H, NG, 8, NT, 128)
    x5 = jnp.transpose(x5, (0, 1, 3, 2, 4))
    x3 = x5.reshape(H, Q, 128)
    xp = x5.reshape(H // 2, 2, NG * NT, 8, 128)
    w2t = jnp.transpose(w2)
    par = jnp.concatenate([
        jnp.pad(grn_gamma.reshape(1, E), ((0, 0), (0, 512 - E))),
        jnp.pad(grn_beta.reshape(1, E), ((0, 0), (0, 512 - E))),
        jnp.pad(dw.reshape(9, C), ((0, 5), (0, 512 - C)))], axis=0)

    kern = functools.partial(_kernel, H=H, C=C, E=E, W=W)
    vmem = pl.BlockSpec(memory_space=pltpu.VMEM)
    hbm = pl.BlockSpec(memory_space=pl.ANY)
    out = pl.pallas_call(
        kern,
        in_specs=[hbm, hbm, vmem, vmem, vmem],
        out_specs=hbm,
        out_shape=jax.ShapeDtypeStruct((H, Q, 128), jnp.bfloat16),
        scratch_shapes=[
            pltpu.VMEM((NB * (TH - len(RC)) - GLESS, E // 2, W), u32),
            pltpu.VMEM((E, 128), f32),
            pltpu.VMEM((E // 2, C), u32),
            pltpu.VMEM((C // 2, E), u32),
            pltpu.VMEM((C, 128), f32),
            pltpu.VMEM((C, 128), f32),
            pltpu.VMEM((NG, 8, 128), u32),
            pltpu.VMEM((NG, 8, 128), u32),
            pltpu.VMEM((NR, 2, Q, 128), u32),
            pltpu.VMEM((NR, 2, C // 2, W), u32),
            pltpu.SemaphoreType.DMA((2, 2)),
            pltpu.SemaphoreType.DMA((3,)),
            pltpu.SemaphoreType.DMA((2,)),
        ],
        compiler_params=pltpu.CompilerParams(
            vmem_limit_bytes=128 * 1024 * 1024,
            disable_bounds_checks=True,
        ),
        name="convnext_block",
    )(xp, x3, par, w1, w2t)
    out = jnp.transpose(out.reshape(H, NG, NT, 8, 128), (0, 1, 3, 2, 4)).reshape(H, C, W)
    return jnp.transpose(out, (0, 2, 1))[None]
```

```python
import functools
import math

import jax
import jax.numpy as jnp
import jax.experimental.pallas as pl
import jax.experimental.pallas.tpu as pltpu

_K0 = math.sqrt(2.0 / math.pi)
_K1 = 0.044715 * _K0
_ALPHA = _K1 ** (1.0 / 3.0)
_KP = _K0 / _ALPHA
_GS = 2.0 * _ALPHA

f32 = jnp.float32
bf16 = jnp.bfloat16
u32 = jnp.uint32

NP = 8
NR = 4
TH = 8
RC = (1, 2, 3)
CH = 64
P2 = 'r0002,r0002,r0002,r0002,x33,r0002,y2,a,z,b,c'
NODMA2 = 0
SLOTMODE = 0
LNLOG = 1
MERGE = 0
CH2 = 192
GLINK = 0
CSPLIT = 0
GLESS = 0
N1 = 256 // NP
N2 = 64
DIST = [4]*12
DIST0 = [0,0]+[4]*8+[8,8]
DISTL = [8,8]+[4]*8+[0,0]

_TAPS = [(0, 0), (0, 1), (0, 2), (1, 0), (1, 2), (2, 0), (2, 1), (2, 2)]


def _tree_sum(vs):
    vs = list(vs)
    while len(vs) > 1:
        nxt = [vs[i] + vs[i + 1] for i in range(0, len(vs) - 1, 2)]
        if len(vs) % 2:
            nxt.append(vs[-1])
        vs = nxt
    return vs[0]


def _sub_allreduce(s):
    s = s + pltpu.roll(s, 4, 0)
    s = s + pltpu.roll(s, 2, 0)
    s = s + pltpu.roll(s, 1, 0)
    return s


def _layernorm_tile(o, C, scale):
    m = _sub_allreduce(_tree_sum(o)) * (1.0 / C)
    d = [t - m for t in o]
    v = _sub_allreduce(_tree_sum([t * t for t in d]))
    if LNLOG:
        r = jnp.exp2(jnp.log(v + C * 1e-5) * (-0.5 * math.log2(math.e)) + scale)
    else:
        r = jax.lax.rsqrt(v + C * 1e-5) * scale
    return jnp.concatenate([t * r for t in d], axis=0).astype(bf16)


def _layernorm_pair(o0, o1, C, lscale):
    if MERGE == 0:
        return _layernorm_tile(o0, C, lscale), _layernorm_tile(o1, C, lscale)
    even = (jax.lax.broadcasted_iota(jnp.int32, (8, 128), 0) & 1) == 0

    def reduce2(a, b):
        s = jnp.where(even, a, b) + pltpu.roll(jnp.where(even, b, a), 7, 0)
        s = s + pltpu.roll(s, 2, 0)
        return s + pltpu.roll(s, 4, 0)

    def split2(s):
        sr = pltpu.roll(s, 1, 0)
        return jnp.where(even, s, sr), jnp.where(even, sr, s)

    if MERGE == 2:
        m0 = _sub_allreduce(_tree_sum(o0)) * (1.0 / C)
        m1 = _sub_allreduce(_tree_sum(o1)) * (1.0 / C)
    else:
        m0, m1 = split2(reduce2(_tree_sum(o0), _tree_sum(o1)) * (1.0 / C))
    d0 = [t - m0 for t in o0]
    d1 = [t - m1 for t in o1]
    v = reduce2(_tree_sum([t * t for t in d0]), _tree_sum([t * t for t in d1]))
    if LNLOG:
        r = jnp.exp2(jnp.log(v + C * 1e-5) * (-0.5 * math.log2(math.e)) + lscale)
    else:
        r = jax.lax.rsqrt(v + C * 1e-5) * lscale
    r0, r1 = split2(r)
    return (jnp.concatenate([t * r0 for t in d0], axis=0).astype(bf16),
            jnp.concatenate([t * r1 for t in d1], axis=0).astype(bf16))


def _gelu2(h):
    return h * (1.0 + jnp.tanh(h * (h * h + _KP)))


def _kernel(xp_hbm, x_hbm, dw_hbm, w1_hbm, w2t_hbm, gam_hbm, bet_hbm,
            o_hbm,
            g_s, acc_s, w1t_s, w2s_s, dwc_s, bias_s, l1_s, l2_s, lr_s, y_s, z_s, w2f_s, gb_s,
            sem_c, sem_x, sem_o, sem_p,
            *, H, C, E, W):
    NB1 = H // (2 * NP)
    NB = H // TH
    NG = C // 8
    NT = W // 128
    NS = NG * NT // 2
    NCH = E // CH
    res_rows = [r for r in range(TH) if r not in RC]
    NRES = len(res_rows)
    ln_scale = _ALPHA * math.sqrt(C)
    ln_off = 0.0
    if LNLOG:
        ln_scale = math.log2(ln_scale)
        ln_off = -1000.0

    g_b = g_s.bitcast(bf16)
    y_b = y_s.bitcast(bf16)
    lane = jax.lax.broadcasted_iota(jnp.int32, (8, 128), 1)
    sub = jax.lax.broadcasted_iota(jnp.int32, (8, 128), 0)
    zero_u = jnp.zeros((8, 128), u32)

    pend = []

    def linked(u):
        due = [v for (n, v) in pend if n <= 1]
        pend[:] = [(n - 1, v) for (n, v) in pend if n > 1]
        if not due:
            return u
        z = jnp.full((8, 128), z_s[0], jnp.int32).astype(u32)
        dep = due[0]
        for v in due[1:]:
            dep = dep | v
        dep = (dep & z)[:, 0:u.shape[1]] if u.shape[1] <= 128 else jnp.concatenate(
            [dep & z, jnp.zeros((8, u.shape[1] - 128), u32)], axis=1)
        return jnp.concatenate([u[0:8] | dep, u[8:]], axis=0)

    def mm1_raw(y, c, ch=CH):
        lhs = pltpu.bitcast(linked(w1t_s[c * ch // 2:(c + 1) * ch // 2, :]), bf16)
        return jnp.dot(lhs, y, preferred_element_type=f32)

    def setup(dwb_s, dw_ref, w1_ref, w2t_ref, gam_ref, bet_ref):
        w2f_s[0:C // 2, :] = pltpu.bitcast(w2t_ref[...], u32)
        gb_s[...] = jnp.zeros(gb_s.shape, f32)
        gb_s[0:1, 0:E] = gam_ref[...].astype(f32).reshape(1, E)
        gb_s[1:2, 0:E] = bet_ref[...].astype(f32).reshape(1, E)
        acc_s[...] = jnp.zeros(acc_s.shape, f32)
        w1t_s[...] = pltpu.bitcast(jnp.transpose(w1_ref[...].astype(f32)).astype(bf16), u32)
        rows = jax.lax.broadcasted_iota(jnp.int32, (C, C), 0)
        cols = jax.lax.broadcasted_iota(jnp.int32, (C, C), 1)
        eye = rows == cols
        for i in range(3):
            for j in range(3):
                d = dw_ref[i, j:j + 1, :].astype(f32)
                col = jnp.sum(jnp.where(eye, d, 0.0), axis=1, keepdims=True)
                dwb_s[i * 3 + j] = jnp.broadcast_to(col, (C, 128))
        r16 = jax.lax.broadcasted_iota(jnp.int32, (16, 128), 0)
        c16 = jax.lax.broadcasted_iota(jnp.int32, (16, 128), 1)
        kv = c16 // 16
        kb = c16 % 16
        k_row = 2 * (kv // 3) + kb // 8 - r16 // 8
        k_j = kv % 3
        for cg in range(NG):
            l1 = jnp.zeros((16, 128), f32)
            l2 = jnp.zeros((16, 128), f32)
            for i in range(3):
                for j in range(3):
                    w8 = dwb_s[i * 3 + j, cg * 8:cg * 8 + 8, :]
                    w16 = jnp.concatenate([w8, w8], axis=0)
                    hit = (kb % 8 == r16 % 8) & (k_row == i) & (k_j == j) & (kv < 6)
                    l1 = jnp.where(hit, w16, l1)
                    if (i, j) in _TAPS:
                        l2 = jnp.where(c16 == r16 + 16 * _TAPS.index((i, j)), w16, l2)
            l1_s[cg] = pltpu.bitcast(l1.astype(bf16), u32)
            l2_s[cg] = pltpu.bitcast(l2.astype(bf16), u32)
        dwc_s[...] = dwb_s[4]
        lr_s[...] = jnp.zeros(lr_s.shape, u32)
        y_s[...] = jnp.zeros(y_s.shape, u32)
        z_s[0] = 0

    def gelu_acc(h, c, gidx):
        g = _gelu2(h)
        g2 = g * g
        acc_s[c * CH:(c + 1) * CH, :] += _tree_sum(
            [g2[:, k * 128:(k + 1) * 128] for k in range(NT)])
        if gidx is not None:
            g_b.at[gidx][c * CH:(c + 1) * CH, :] = g.astype(bf16)

    def gindex(blk, r):
        if r % TH not in res_rows:
            return None
        b = blk * (2 * NP // TH) + r // TH
        if r < 0:
            b = jnp.maximum(b, 0)
        return b * NRES + res_rows.index(r % TH)

    def pass1(cbuf, zb_s, cl_s):
        cu = cbuf.bitcast(u32)

        def c_copies(blk, slot):
            return [
                pltpu.make_async_copy(xp_hbm.at[pl.ds(blk * NP - 1, NP), 1],
                                      cbuf.at[slot, :, :, pl.ds(0, 8), :], sem_c.at[slot, 0]),
                pltpu.make_async_copy(xp_hbm.at[pl.ds(blk * NP, NP), 0],
                                      cbuf.at[slot, :, :, pl.ds(8, 8), :], sem_c.at[slot, 1]),
            ]

        def last_copy(slot):
            return pltpu.make_async_copy(xp_hbm.at[NB1 * NP - 1, 1],
                                         cbuf.at[slot, 0, :, pl.ds(0, 8), :], sem_c.at[slot, 0])

        def load_params(dwb_s, *bufs):
            cps = [pltpu.make_async_copy(src, dst, sem_p.at[n]) for n, (src, dst) in
                   enumerate(zip((dw_hbm, w1_hbm, w2t_hbm, gam_hbm, bet_hbm), bufs))]
            for c in cps:
                c.start()
            pltpu.make_async_copy(xp_hbm.at[pl.ds(0, NP), 0],
                                  cbuf.at[0, :, :, pl.ds(8, 8), :], sem_c.at[0, 1]).start()
            pltpu.make_async_copy(xp_hbm.at[pl.ds(0, NP - 1), 1],
                                  cbuf.at[0, pl.ds(1, NP - 1), :, pl.ds(0, 8), :], sem_c.at[0, 0]).start()
            zb_s[...] = jnp.zeros(zb_s.shape, bf16)
            pltpu.make_async_copy(zb_s, cbuf.at[0, 0, :, pl.ds(0, 8), :], sem_c.at[0, 0]).start()
            for c in cps:
                c.wait()
            setup(dwb_s, *bufs)

        pl.run_scoped(
            load_params,
            pltpu.VMEM((9, C, 128), f32),
            pltpu.VMEM((3, 3, C), bf16),
            pltpu.VMEM((C, E), bf16),
            pltpu.VMEM((C, E), bf16),
            pltpu.VMEM((E,), bf16),
            pltpu.VMEM((E,), bf16),
        )
        cl_s[...] = jnp.zeros(cl_s.shape, u32)

        def a1(slot, q):
            for cg in range(NG):
                t = [cu[slot, q, cg * NT + k] for k in range(NT)]
                for k in range(NT):
                    lo = (cg * NT + k) * 8
                    if q == NP - 1:
                        cl_s[lo:lo + 8, :] = t[k]
                    lsrc = t[k - 1] if k > 0 else zero_u
                    rsrc = t[k + 1] if k < NT - 1 else zero_u
                    lr_s[q % NR, 0, lo:lo + 8, :] = pltpu.roll(jnp.where(lane == 127, lsrc, t[k]), 1, 1)
                    lr_s[q % NR, 1, lo:lo + 8, :] = pltpu.roll(jnp.where(lane == 0, rsrc, t[k]), 127, 1)

        def conv_pair_dot(slot, j, cg, k):
            n = cg * NT + k
            parts = []
            for q in (j, j + 1):
                c = cu[slot, q, n] if q >= 0 else cl_s[8 * n:8 * n + 8, :]
                parts += [lr_s[q % NR, 0, 8 * n:8 * n + 8, :], c, lr_s[q % NR, 1, 8 * n:8 * n + 8, :]]
            wt = pltpu.bitcast(jnp.concatenate(parts, axis=0), bf16)
            lhs = pltpu.bitcast(l1_s[cg, :, 0:96], bf16)
            return jnp.dot(lhs, wt, preferred_element_type=f32)

        def b_and_c(slot, j, scale, yslot, gidx, dist):
            order = [(k, cg) for k in range(NT) for cg in range(NG)]
            o = {}
            pos = 0
            for n in range(2 * NCH):
                gelu_acc(mm1_raw(y_b[yslot, n // NCH], n % NCH), n % NCH, gidx[n // NCH])
                for (k, cg) in order[pos:pos + dist[n]]:
                    o[cg] = conv_pair_dot(slot, j, cg, k)
                    if cg == NG - 1:
                        yt = _layernorm_pair([o[q][0:8] for q in range(NG)],
                                             [o[q][8:16] for q in range(NG)], C, scale)
                        for hh in range(2):
                            y_b.at[j % NR, hh][:, k * 128:(k + 1) * 128] = yt[hh]
                pos += dist[n]

        def body(i, carry):
            slot = i & 1
            for c in c_copies(1, slot):
                c.wait()

            @pl.when(i + 1 < NB1)
            def _():
                for c in c_copies(i + 1, 1 - slot):
                    c.start()

            @pl.when(i + 1 == NB1)
            def _():
                last_copy(1 - slot).start()

            for j in range(-1, NP - 1):
                scale = jnp.where(i > 0, ln_scale, ln_off) if j == -1 else ln_scale
                a1(slot, j + 1)
                jc = j - 2
                b_and_c(slot, j, scale, jc % NR, [gindex(i, 2 * jc), gindex(i, 2 * jc + 1)],
                        DIST0 if j == -1 else (DISTL if j == NP - 2 else DIST))
            return carry

        jax.lax.fori_loop(0, N1, body, 0)

        slot = NB1 % 2
        last_copy(slot).wait()
        cbuf[slot, 0, :, pl.ds(8, 8), :] = jnp.zeros((NG * NT, 8, 128), bf16)
        a1(slot, 0)
        b_and_c(slot, -1, ln_scale, (-3) % NR, [gindex(NB1, -6), gindex(NB1, -5)], DIST0)

    pl.run_scoped(
        pass1,
        pltpu.VMEM((2, NP, NG * NT, 16, 128), bf16),
        pltpu.VMEM((NG * NT, 8, 128), bf16),
        pltpu.VMEM((NG * NT * 8, 128), u32),
    )

    def pass2(xbuf, obuf, gt_s):
        xu = xbuf.bitcast(u32)
        gt_b = gt_s.bitcast(bf16)

        def x_copy(blk, slot):
            return pltpu.make_async_copy(x_hbm.at[pl.ds(blk * TH, TH)], xbuf.at[slot], sem_x.at[slot])

        def o_copy(blk, slot):
            return pltpu.make_async_copy(obuf.at[slot], o_hbm.at[pl.ds(blk * TH, TH)], sem_o.at[slot])

        x_copy(0, 0).start()
        x_copy(1, 1).start()

        for jc in (-2, -1):
            for n in range(2 * NCH):
                gelu_acc(mm1_raw(y_b[jc % NR, n // NCH], n % NCH), n % NCH,
                         gindex(NB1, 2 * jc + n // NCH))

        ssq = jnp.sum(jnp.transpose(acc_s[...]), axis=0, keepdims=True)
        gx = jnp.sqrt(ssq * (1.0 / (_GS * _GS)) + 1e-6)
        nx = gx / (jnp.sum(gx, axis=1, keepdims=True) * (1.0 / E) + 1e-6)
        par = gb_s[...]
        sc = (par[0:1, 0:E] * nx + 1.0) * (1.0 / _GS)
        w2 = pltpu.bitcast(w2f_s[0:C // 2, :], bf16).astype(f32)
        w2s_s[0:C // 2, :] = pltpu.bitcast((w2 * sc).astype(bf16), u32)
        b = jnp.sum(w2 * par[1:2, 0:E], axis=1, keepdims=True)
        bias_s[...] = jnp.broadcast_to(b, (C, 128))

        def xs_idx(r, v, s):
            n = 2 * (r - RC[0] + 1) + v
            return (n // 4, (n % 4) // 2, pl.ds((n % 2) * NS * 8 + 8 * s, 8), slice(None))

        def shift_rows(slot, rows):
            for s in [2 * cg + pp for pp in range(NT // 2) for cg in range(NG)]:
              for r in rows:
                a = xu[slot, r, 8 * s:8 * s + 8, :]
                bl = xu[slot, r, 8 * s - 4:8 * s + 4, :] if s > 0 else pltpu.roll(a, 4, 0)
                br = xu[slot, r, 8 * s + 4:8 * s + 12, :] if s < NS - 1 else pltpu.roll(a, 4, 0)
                if s % 2 == 0:
                    bl = jnp.where(sub < 4, zero_u, bl)
                else:
                    br = jnp.where(sub >= 4, zero_u, br)
                lr_s[xs_idx(r, 0, s)] = pltpu.roll(jnp.where(lane == 127, bl, a), 1, 1)
                lr_s[xs_idx(r, 1, s)] = pltpu.roll(jnp.where(lane == 0, br, a), 127, 1)

        def conv_dot(slot, r, s):
            cg = s // 2
            parts = []
            for (i, j) in _TAPS:
                rr = r + i - 1
                if j == 1:
                    parts.append(xu[slot, rr, 8 * s:8 * s + 8, :])
                else:
                    parts.append(lr_s[xs_idx(rr, j // 2, s)])
            wt = pltpu.bitcast(jnp.concatenate(parts, axis=0), bf16)
            lhs = pltpu.bitcast(l2_s[cg], bf16)
            p = jnp.dot(lhs, wt, preferred_element_type=f32)
            xc = pltpu.bitcast(xu[slot, r, 8 * s:8 * s + 8, :], bf16).astype(f32)
            w8 = dwc_s[cg * 8:cg * 8 + 8, :]
            return [p[0:8] + xc[0:8] * w8, p[8:16] + xc[8:16] * w8]

        def conv_ln_gen(slot, r, n):
            cnt = 0
            for pp in range(NT // 2):
                o = []
                for cg in range(NG):
                    o.append(conv_dot(slot, r, 2 * cg + pp))
                    cnt += 1
                    if cg == NG - 1:
                        yt = _layernorm_pair([o[q][0] for q in range(NG)],
                                             [o[q][1] for q in range(NG)], C, ln_scale)
                        for h in range(2):
                            k = 2 * pp + h
                            y_b.at[n // 2, n % 2][:, k * 128:(k + 1) * 128] = yt[h]
                    if cnt % 4 == 0:
                        yield

        def stage_d(slot, oslot, r, g, gen, per):
            lhs = pltpu.bitcast(linked(w2s_s[0:C // 2, :]), bf16)
            p = []
            full = sum(per[:NT - 1]) == 0
            if full:
                pf = jnp.dot(lhs, g, preferred_element_type=f32)
            for k in range(NT):
                if full:
                    p.append(pf[:, k * 128:(k + 1) * 128])
                else:
                    p.append(jnp.dot(lhs, g[:, k * 128:(k + 1) * 128], preferred_element_type=f32))
                for _ in range(per[k]):
                    next(gen)
                if k % 2 == 1:
                    pp = k // 2
                    for cg in range(NG):
                        b8 = bias_s[cg * 8:cg * 8 + 8, :]
                        s = 2 * cg + pp
                        xr = pltpu.bitcast(xu[slot, r, 8 * s:8 * s + 8, :], bf16).astype(f32)
                        v = [xr[8 * h:8 * h + 8] + (p[2 * pp + h][cg * 8:cg * 8 + 8] + b8)
                             for h in range(2)]
                        obuf[oslot, r, 16 * s:16 * s + 16, :] = jnp.concatenate(v, axis=0).astype(bf16)

        def body(i, slot):
            oslot = i & 1
            if SLOTMODE == 1:
                slot = jax.lax.rem(i, 3)
            if SLOTMODE == 2:
                slot = i & 1
            if SLOTMODE == 3:
                slot = (i & 1) + 1
            if SLOTMODE == 5:
                slot = (i & 1) ^ 1
            if SLOTMODE == 6:
                slot = 2 - (i & 1)
            if SLOTMODE == 7:
                slot = (i >> 1) & 1
            if SLOTMODE == 4:
                slot = (i & 1) * 2
            if not NODMA2 & 1:
                x_copy(i, slot).wait()

            if not NODMA2 & 2:
                @pl.when(i >= 2)
                def _():
                    o_copy(i - 2, oslot).wait()

            if not NODMA2 & 1:
                @pl.when(i + 2 < NB)
                def _():
                    x_copy(i + 2, jnp.where(slot == 0, 2, slot - 1)).start()

            res = list(res_rows)
            pend.clear()

            def c_row(n, gen, per):
                if sum(per) == 0 and not CSPLIT:
                    lhs = pltpu.bitcast(w1t_s[...], bf16)
                    return [_gelu2(jnp.dot(lhs, y_b[n // 2, n % 2], preferred_element_type=f32))]
                out = []
                for c in range(E // CH2):
                    out.append(_gelu2(mm1_raw(y_b[n // 2, n % 2], c, CH2)))
                    if GLINK:
                        pend.append((GLINK, pltpu.bitcast(out[-1][CH2 - 8:CH2, W - 128:W], u32)))
                    for _ in range(per[c]):
                        next(gen)
                return out

            shift_rows(slot, range(RC[0] - 1, RC[0] + 2))
            for r in range(RC[0] + 2, RC[-1] + 2):
                shift_rows(slot, [r])
            gens = [conv_ln_gen(slot, r, n) for n, r in enumerate(RC)]

            def chain():
                for g_ in gens:
                    yield from g_
            ch = chain()
            for tok in P2.split(','):
                op = tok[0]
                per = [int(c) for c in tok[1:]] + [0] * 8
                if op == 'r':
                    r = res.pop(0)
                    stage_d(slot, oslot, r, g_b[i * NRES + res_rows.index(r)], ch, per)
                elif op in 'xyz':
                    n = 'xyz'.index(op)
                    gl = c_row(n, ch, per)
                    lo = 0
                    for gg in gl:
                        gt_b.at[n][lo:lo + gg.shape[0], :] = gg.astype(bf16)
                        lo += gg.shape[0]
                else:
                    n = 'abc'.index(op)
                    stage_d(slot, oslot, RC[n], gt_b[n], ch, per)
            assert not res and next(ch, 'done') == 'done'
            pend.clear()
            if not NODMA2 & 2:
                o_copy(i, oslot).start()
            return jnp.where(slot == 2, 0, slot + 1)

        jax.lax.fori_loop(0, N2, body, 0)
        if NODMA2 & 2:
            o_copy(0, 0).start()
            o_copy(1, 1).start()
        o_copy(N2 - 2, N2 % 2).wait()
        o_copy(N2 - 1, (N2 - 1) % 2).wait()
        if NODMA2 & 1:
            x_copy(0, 0).wait()
            x_copy(1, 1).wait()
        if N2 < NB:
            x_copy(N2, N2 % 3).wait()
        if N2 + 1 < NB:
            x_copy(N2 + 1, (N2 + 1) % 3).wait()

    pl.run_scoped(
        pass2,
        pltpu.VMEM((3, TH, NS * 16, 128), bf16),
        pltpu.VMEM((2, TH, NS * 16, 128), bf16),
        pltpu.VMEM((len(RC), E // 2, W), u32),
    )


@jax.jit
def pallas_standalone__modern_conv_block_convnext_v2__vision_kernel(
    x: jax.Array,
    dw: jax.Array,
    w1: jax.Array,
    w2: jax.Array,
    grn_gamma: jax.Array,
    grn_beta: jax.Array,
):
    B, H, W, C = x.shape
    E = w1.shape[1]
    assert B == 1
    NB = H // TH
    NG = C // 8
    NT = W // 128
    Q = NG * NT * 8
    x5 = jnp.transpose(x[0], (0, 2, 1)).reshape(H, NG, 8, NT, 128)
    x5 = jnp.transpose(x5, (0, 1, 3, 2, 4))
    x3 = x5.reshape(H, Q, 128)
    xp = x5.reshape(H // 2, 2, NG * NT, 8, 128)
    w2t = jnp.transpose(w2)

    kern = functools.partial(_kernel, H=H, C=C, E=E, W=W)
    hbm = pl.BlockSpec(memory_space=pl.ANY)
    out = pl.pallas_call(
        kern,
        in_specs=[hbm] * 7,
        out_specs=hbm,
        out_shape=jax.ShapeDtypeStruct((H, Q, 128), jnp.bfloat16),
        scratch_shapes=[
            pltpu.VMEM((NB * (TH - len(RC)) - GLESS, E // 2, W), u32),
            pltpu.VMEM((E, 128), f32),
            pltpu.VMEM((E // 2, C), u32),
            pltpu.VMEM((C // 2, E), u32),
            pltpu.VMEM((C, 128), f32),
            pltpu.VMEM((C, 128), f32),
            pltpu.VMEM((NG, 8, 128), u32),
            pltpu.VMEM((NG, 8, 128), u32),
            pltpu.VMEM((NR, 2, Q, 128), u32),
            pltpu.VMEM((NR, 2, C // 2, W), u32),
            pltpu.SMEM((1,), jnp.int32),
            pltpu.VMEM((64, E), u32),
            pltpu.VMEM((8, 512), f32),
            pltpu.SemaphoreType.DMA((2, 2)),
            pltpu.SemaphoreType.DMA((3,)),
            pltpu.SemaphoreType.DMA((2,)),
            pltpu.SemaphoreType.DMA((5,)),
        ],
        compiler_params=pltpu.CompilerParams(
            vmem_limit_bytes=128 * 1024 * 1024,
            disable_bounds_checks=True,
        ),
        name="convnext_block",
    )(xp, x3, dw, w1, w2t, grn_gamma, grn_beta)
    out = jnp.transpose(out.reshape(H, NG, NT, 8, 128), (0, 1, 3, 2, 4)).reshape(H, C, W)
    return jnp.transpose(out, (0, 2, 1))[None]
```

```python
import functools
import math

import jax
import jax.numpy as jnp
import jax.experimental.pallas as pl
import jax.experimental.pallas.tpu as pltpu

_K0 = math.sqrt(2.0 / math.pi)
_K1 = 0.044715 * _K0
_ALPHA = _K1 ** (1.0 / 3.0)
_KP = _K0 / _ALPHA
_GS = 2.0 * _ALPHA

f32 = jnp.float32
bf16 = jnp.bfloat16
u32 = jnp.uint32

NP = 8
NR = 4
TH = 8
RC = (1, 2, 3)
CH = 64
CH2 = 192
P2 = 'r0101,r0101,r1010,r1010,r1111,x,y,a,z,b,c'
RORD = [5,6,7,0,4]
PG = 3
LDIST = 2
CSPLIT = 0
GLESS = 0
N2 = 64
DIST = [4]*12
DIST0 = [0,0]+[4]*8+[8,8]
DISTL = [8,8]+[4]*8+[0,0]


def _tree_sum(vs):
    vs = list(vs)
    while len(vs) > 1:
        nxt = [vs[i] + vs[i + 1] for i in range(0, len(vs) - 1, 2)]
        if len(vs) % 2:
            nxt.append(vs[-1])
        vs = nxt
    return vs[0]


def _sub_allreduce(s):
    s = s + pltpu.roll(s, 4, 0)
    s = s + pltpu.roll(s, 2, 0)
    s = s + pltpu.roll(s, 1, 0)
    return s


def _layernorm_tile(o, C, log2_scale):
    m = _sub_allreduce(_tree_sum(o)) * (1.0 / C)
    d = [t - m for t in o]
    v = _sub_allreduce(_tree_sum([t * t for t in d]))
    r = jnp.exp2(jnp.log(v + C * 1e-5) * (-0.5 * math.log2(math.e)) + log2_scale)
    return jnp.concatenate([t * r for t in d], axis=0).astype(bf16)


def _gelu2(h):
    return h * (1.0 + jnp.tanh(h * (h * h + _KP)))


def _kernel(xp_hbm, x_hbm, dw_hbm, w1_hbm, w2t_hbm, gam_hbm, bet_hbm,
            o_hbm,
            g_s, xc_s, lr_s, y_s, cl_s, acc_s, w1t_s, w2s_s, w2f_s, bias_s, l1_s, gb_s, dwr_s, z_s,
            sem_c, sem_x, sem_o, sem_p,
            *, H, C, E, W):
    NB1 = H // (2 * NP)
    NB = H // TH
    NG = C // 8
    NT = W // 128
    NS = NG * NT // 2
    NV = NG * NT
    NCH = E // CH
    res_rows = [r for r in range(TH) if r not in RC]
    NRES = len(res_rows)
    ln_scale = math.log2(_ALPHA * math.sqrt(C))

    g_b = g_s.bitcast(bf16)
    y_b = y_s.bitcast(bf16)
    xu = xc_s.bitcast(u32)
    lane = jax.lax.broadcasted_iota(jnp.int32, (8, 128), 1)
    zero_u = jnp.zeros((8, 128), u32)
    zero_f = jnp.zeros((8, 128), f32)

    def wtap_idx(t):
        return (2 + t // 8, (t % 8) // 4)

    def build_taps():
        rows = jax.lax.broadcasted_iota(jnp.int32, (C, 128), 0)
        cols = jax.lax.broadcasted_iota(jnp.int32, (C, 128), 1)
        for t in range(9):
            col = jnp.sum(jnp.where(rows == cols, dwr_s[t:t + 1, :], 0.0), axis=1, keepdims=True)
            a, b = wtap_idx(t)
            lr_s[a, b, (t % 4) * C:(t % 4 + 1) * C, :] = pltpu.bitcast(
                jnp.broadcast_to(col, (C, 128)), u32)

    def wtap(i, j, cg):
        t = i * 3 + j
        lo = (t % 4) * C + cg * 8
        a, b = wtap_idx(t)
        return pltpu.bitcast(lr_s[a, b, lo:lo + 8, :], f32)

    pend = []

    def linked(u):
        due = [v for (n, v) in pend if n <= 1]
        pend[:] = [(n - 1, v) for (n, v) in pend if n > 1]
        if not due:
            return u
        dep = due[0]
        for v in due[1:]:
            dep = dep | v
        dep = dep & jnp.full((8, 128), z_s[0], jnp.int32).astype(u32)
        if u.shape[1] <= 128:
            dep = dep[:, 0:u.shape[1]]
        else:
            dep = jnp.concatenate([dep, jnp.zeros((8, u.shape[1] - 128), u32)], axis=1)
        return jnp.concatenate([u[0:8] | dep, u[8:]], axis=0)

    def mm1_raw(y, c, ch):
        lhs = pltpu.bitcast(linked(w1t_s[c * ch // 2:(c + 1) * ch // 2, :]), bf16)
        return jnp.dot(lhs, y, preferred_element_type=f32)

    def gelu_acc(h, c, gidx):
        g = _gelu2(h)
        g2 = g * g
        acc_s[c * CH:(c + 1) * CH, :] += _tree_sum(
            [g2[:, k * 128:(k + 1) * 128] for k in range(NT)])
        if gidx is not None:
            g_b.at[gidx][c * CH:(c + 1) * CH, :] = g.astype(bf16)

    def gindex(blk, r):
        if r % TH not in res_rows:
            return None
        b = blk * (2 * NP // TH) + r // TH
        if r < 0:
            b = jnp.maximum(b, 0)
        return b * NRES + res_rows.index(r % TH)

    def c_copies(blk, slot):
        return [
            pltpu.make_async_copy(xp_hbm.at[pl.ds(blk * NP - 1, NP), 1],
                                  xc_s.at[slot, :, :, pl.ds(0, 8), :], sem_c.at[slot, 0]),
            pltpu.make_async_copy(xp_hbm.at[pl.ds(blk * NP, NP), 0],
                                  xc_s.at[slot, :, :, pl.ds(8, 8), :], sem_c.at[slot, 1]),
        ]

    def last_copy(slot):
        return pltpu.make_async_copy(xp_hbm.at[NB1 * NP - 1, 1],
                                     xc_s.at[slot, 0, :, pl.ds(0, 8), :], sem_c.at[slot, 0])

    def setup(dw_ref, w1_ref, w2t_ref, gam_ref, bet_ref):
        bufs = (dw_ref, w1_ref, w2t_ref, gam_ref, bet_ref)
        cps = [pltpu.make_async_copy(src, dst, sem_p.at[n]) for n, (src, dst) in
               enumerate(zip((dw_hbm, w1_hbm, w2t_hbm, gam_hbm, bet_hbm), bufs))]
        for c in cps:
            c.start()
        pltpu.make_async_copy(xp_hbm.at[pl.ds(0, NP), 0],
                              xc_s.at[0, :, :, pl.ds(8, 8), :], sem_c.at[0, 1]).start()
        pltpu.make_async_copy(xp_hbm.at[pl.ds(0, NP - 1), 1],
                              xc_s.at[0, pl.ds(1, NP - 1), :, pl.ds(0, 8), :], sem_c.at[0, 0]).start()
        xc_s[1, 0, :, pl.ds(0, 8), :] = jnp.zeros((NV, 8, 128), bf16)
        pltpu.make_async_copy(xc_s.at[1, 0, :, pl.ds(0, 8), :],
                              xc_s.at[0, 0, :, pl.ds(0, 8), :], sem_c.at[0, 0]).start()
        for c in cps:
            c.wait()

        z_s[0] = 0
        acc_s[...] = jnp.zeros(acc_s.shape, f32)
        cl_s[...] = jnp.zeros(cl_s.shape, u32)
        y_s[...] = jnp.zeros(y_s.shape, u32)
        gb_s[...] = jnp.zeros(gb_s.shape, f32)
        dwr_s[...] = jnp.zeros(dwr_s.shape, f32)
        gb_s[0:1, 0:E] = gam_ref[...].astype(f32).reshape(1, E)
        gb_s[1:2, 0:E] = bet_ref[...].astype(f32).reshape(1, E)
        w2f_s[0:C // 2, :] = pltpu.bitcast(w2t_ref[...], u32)
        w1t_s[...] = pltpu.bitcast(jnp.transpose(w1_ref[...].astype(f32)).astype(bf16), u32)
        for i in range(3):
            for j in range(3):
                dwr_s[i * 3 + j:i * 3 + j + 1, 0:C] = dw_ref[i, j:j + 1, :].astype(f32)
        build_taps()
        r16 = jax.lax.broadcasted_iota(jnp.int32, (16, 128), 0)
        c16 = jax.lax.broadcasted_iota(jnp.int32, (16, 128), 1)
        kv = c16 // 16
        kb = c16 % 16
        k_row = 2 * (kv // 3) + kb // 8 - r16 // 8
        k_j = kv % 3
        for cg in range(NG):
            l1 = jnp.zeros((16, 128), f32)
            for i in range(3):
                for j in range(3):
                    w8 = wtap(i, j, cg)
                    hit = (kb % 8 == r16 % 8) & (k_row == i) & (k_j == j) & (kv < 6)
                    l1 = jnp.where(hit, jnp.concatenate([w8, w8], axis=0), l1)
            l1_s[cg] = pltpu.bitcast(l1.astype(bf16), u32)
        lr_s[NR - 1] = jnp.zeros(lr_s.shape[1:], u32)

    pl.run_scoped(
        setup,
        pltpu.VMEM((3, 3, C), bf16),
        pltpu.VMEM((C, E), bf16),
        pltpu.VMEM((C, E), bf16),
        pltpu.VMEM((E,), bf16),
        pltpu.VMEM((E,), bf16),
    )

    def a1(slot, q):
        for cg in range(NG):
            t = [xu[slot, q, cg * NT + k] for k in range(NT)]
            for k in range(NT):
                lo = (cg * NT + k) * 8
                if q == NP - 1:
                    cl_s[lo:lo + 8, :] = t[k]
                lsrc = t[k - 1] if k > 0 else zero_u
                rsrc = t[k + 1] if k < NT - 1 else zero_u
                lr_s[q % NR, 0, lo:lo + 8, :] = pltpu.roll(jnp.where(lane == 127, lsrc, t[k]), 1, 1)
                lr_s[q % NR, 1, lo:lo + 8, :] = pltpu.roll(jnp.where(lane == 0, rsrc, t[k]), 127, 1)

    def conv_pair_dot(slot, j, cg, k):
        n = cg * NT + k
        parts = []
        for q in (j, j + 1):
            c = xu[slot, q, n] if q >= 0 else cl_s[8 * n:8 * n + 8, :]
            parts += [lr_s[q % NR, 0, 8 * n:8 * n + 8, :], c, lr_s[q % NR, 1, 8 * n:8 * n + 8, :]]
        wt = pltpu.bitcast(jnp.concatenate(parts, axis=0), bf16)
        lhs = pltpu.bitcast(l1_s[cg, :, 0:96], bf16)
        return jnp.dot(lhs, wt, preferred_element_type=f32)

    def b_and_c(slot, j, scale, yslot, gidx, dist):
        order = [(k, cg) for k in range(NT) for cg in range(NG)]
        o = {}
        pos = 0
        for n in range(2 * NCH):
            gelu_acc(mm1_raw(y_b[yslot, n // NCH], n % NCH, CH), n % NCH, gidx[n // NCH])
            for (k, cg) in order[pos:pos + dist[n]]:
                o[cg] = conv_pair_dot(slot, j, cg, k)
                if cg == NG - 1:
                    for hh in range(2):
                        yt = _layernorm_tile([o[q][8 * hh:8 * hh + 8] for q in range(NG)], C, scale)
                        y_b.at[j % NR, hh][:, k * 128:(k + 1) * 128] = yt
            pos += dist[n]

    def p1_body(i, carry):
        slot = i & 1
        for c in c_copies(1, slot):
            c.wait()

        @pl.when(i + 1 < NB1)
        def _():
            for c in c_copies(i + 1, 1 - slot):
                c.start()

        @pl.when(i + 1 == NB1)
        def _():
            last_copy(1 - slot).start()

        for j in range(-1, NP - 1):
            scale = jnp.where(i > 0, ln_scale, -1000.0) if j == -1 else ln_scale
            a1(slot, j + 1)
            jc = j - 2
            b_and_c(slot, j, scale, jc % NR, [gindex(i, 2 * jc), gindex(i, 2 * jc + 1)],
                    DIST0 if j == -1 else (DISTL if j == NP - 2 else DIST))
        return carry

    jax.lax.fori_loop(0, NB1, p1_body, 0)

    def xslot(s):
        return xc_s.at[s >> 1, pl.ds((s & 1) * (TH // 2), TH // 2)]

    def x_copy(blk, s):
        return pltpu.make_async_copy(x_hbm.at[pl.ds(blk * (TH // 2), TH // 2)], xslot(s), sem_x.at[s])

    def o_copy(blk, s):
        return pltpu.make_async_copy(xslot(s), o_hbm.at[pl.ds(blk * (TH // 2), TH // 2)], sem_o.at[s])

    dslot = NB1 % 2
    S0 = 2 * (1 - dslot)
    last_copy(dslot).wait()
    x_copy(0, S0).start()
    x_copy(1, S0 + 1).start()
    xc_s[dslot, 0, :, pl.ds(8, 8), :] = jnp.zeros((NV, 8, 128), bf16)
    a1(dslot, 0)
    b_and_c(dslot, -1, ln_scale, (-3) % NR, [gindex(NB1, -6), gindex(NB1, -5)], DIST0)
    for jc in (-2, -1):
        for n in range(2 * NCH):
            gelu_acc(mm1_raw(y_b[jc % NR, n // NCH], n % NCH, CH), n % NCH,
                     gindex(NB1, 2 * jc + n // NCH))

    ssq = jnp.sum(jnp.transpose(acc_s[...]), axis=0, keepdims=True)
    gx = jnp.sqrt(ssq * (1.0 / (_GS * _GS)) + 1e-6)
    nx = gx / (jnp.sum(gx, axis=1, keepdims=True) * (1.0 / E) + 1e-6)
    sc = (gb_s[0:1, 0:E] * nx + 1.0) * (1.0 / _GS)
    w2 = pltpu.bitcast(w2f_s[0:C // 2, :], bf16).astype(f32)
    w2s_s[0:C // 2, :] = pltpu.bitcast((w2 * sc).astype(bf16), u32)
    b = jnp.sum(w2 * gb_s[1:2, 0:E], axis=1, keepdims=True)
    bias_s[...] = jnp.broadcast_to(b, (C, 128))
    build_taps()

    def pass2(gt_s):
        gt_b = gt_s.bitcast(bf16)

        def o_idx(n, k, cg):
            m = (n * NT + k) * NG + cg
            return (m // (2 * NV), (m // NV) % 2, pl.ds((m % NV) * 8, 8), slice(None))

        def p2_body(i, carry):
            s = (i + S0) & 3
            sa, sb = s >> 1, (s & 1) * (TH // 2)
            x_copy(0, s).wait()

            @pl.when(i >= 2)
            def _():
                o_copy(0, (s + 2) & 3).wait()

            @pl.when(i + 2 < NB)
            def _():
                x_copy(i + 2, (s + 2) & 3).start()

            def xrow(r, slab):
                v = pltpu.bitcast(xu[sa, sb + r // 2, (r % 2) * NS + slab], bf16).astype(f32)
                return [v[0:8], v[8:16]]

            def conv_piece(n, cgs):
                outs = []
                for cg in cgs:
                    rows_ = [xrow(r, 2 * cg) + xrow(r, 2 * cg + 1) for r in range(RC[n] - 1, RC[n] + 2)]
                    w = [[wtap(ii, j, cg) for j in range(3)] for ii in range(3)]
                    t = [[rows_[0][k] * w[0][j] + rows_[1][k] * w[1][j] + rows_[2][k] * w[2][j]
                          for k in range(NT)] for j in range(3)]
                    for k in range(NT):
                        lsrc = t[0][k - 1] if k > 0 else zero_f
                        rsrc = t[2][k + 1] if k < NT - 1 else zero_f
                        left = pltpu.roll(jnp.where(lane == 127, lsrc, t[0][k]), 1, 1)
                        right = pltpu.roll(jnp.where(lane == 0, rsrc, t[2][k]), 127, 1)
                        ov = pltpu.bitcast(t[1][k] + left + right, u32)
                        lr_s[o_idx(n, k, cg)] = ov
                        outs.append(ov)
                dep = outs[0]
                for v in outs[1:]:
                    dep = dep | v
                pend.append((LDIST, dep))

            done = [False] * len(RC)

            def pieces():
                for n in range(len(RC)):
                    for c0 in range(0, NG, PG):
                        conv_piece(n, range(c0, c0 + PG))
                        if c0 + PG == NG:
                            done[n] = True
                            for k in range(NT):
                                o = [pltpu.bitcast(lr_s[o_idx(n, k, cg)], f32) for cg in range(NG)]
                                y_b.at[n // 2, n % 2][:, k * 128:(k + 1) * 128] = _layernorm_tile(
                                    o, C, ln_scale)
                        yield

            def stage_d(r, g, gen, per):
                p = []
                full = sum(per[:NT - 1]) == 0
                if full:
                    lhs = pltpu.bitcast(linked(w2s_s[0:C // 2, :]), bf16)
                    pf = jnp.dot(lhs, g, preferred_element_type=f32)
                for k in range(NT):
                    if full:
                        p.append(pf[:, k * 128:(k + 1) * 128])
                    else:
                        lhs = pltpu.bitcast(linked(w2s_s[0:C // 2, :]), bf16)
                        p.append(jnp.dot(lhs, g[:, k * 128:(k + 1) * 128], preferred_element_type=f32))
                    for _ in range(per[k]):
                        next(gen)
                assert all(done[n] for n in range(len(RC)) if abs(RC[n] - r) <= 1)
                for pp in range(NT // 2):
                    for cg in range(NG):
                        b8 = bias_s[cg * 8:cg * 8 + 8, :]
                        slab = 2 * cg + pp
                        xr = xrow(r, slab)
                        v = [xr[h] + (p[2 * pp + h][cg * 8:cg * 8 + 8] + b8) for h in range(2)]
                        xc_s[sa, sb + r // 2, (r % 2) * NS + slab] = jnp.concatenate(
                            v, axis=0).astype(bf16)

            pend.clear()
            res = list(RORD)
            gen = pieces()
            for tok in P2.split(','):
                op = tok[0]
                per = [int(c) for c in tok[1:]] + [0] * 8
                if op == 'r':
                    r = res.pop(0)
                    stage_d(r, g_b[i * NRES + res_rows.index(r)], gen, per)
                elif op in 'xyz':
                    n = 'xyz'.index(op)
                    ch = CH2 if (sum(per) or CSPLIT) else E
                    for c in range(E // ch):
                        gt_b.at[n][c * ch:(c + 1) * ch, :] = _gelu2(
                            mm1_raw(y_b[n // 2, n % 2], c, ch)).astype(bf16)
                        for _ in range(per[c]):
                            next(gen)
                else:
                    n = 'abc'.index(op)
                    stage_d(RC[n], gt_b[n], gen, per)
            assert not res and next(gen, 'done') == 'done'
            pend.clear()
            o_copy(i, s).start()
            return carry

        jax.lax.fori_loop(0, N2, p2_body, 0)
        o_copy(0, (N2 - 2 + S0) & 3).wait()
        o_copy(0, (N2 - 1 + S0) & 3).wait()
        if N2 < NB:
            x_copy(0, (N2 + S0) & 3).wait()
        if N2 + 1 < NB:
            x_copy(0, (N2 + 1 + S0) & 3).wait()

    pl.run_scoped(pass2, pltpu.VMEM((len(RC), E // 2, W), u32))


@jax.jit
def pallas_standalone__modern_conv_block_convnext_v2__vision_kernel(
    x: jax.Array,
    dw: jax.Array,
    w1: jax.Array,
    w2: jax.Array,
    grn_gamma: jax.Array,
    grn_beta: jax.Array,
):
    B, H, W, C = x.shape
    E = w1.shape[1]
    assert B == 1
    NB = H // TH
    NG = C // 8
    NT = W // 128
    NV = NG * NT
    x5 = jnp.transpose(x[0], (0, 2, 1)).reshape(H, NG, 8, NT, 128)
    x5 = jnp.transpose(x5, (0, 1, 3, 2, 4))
    xn = x5.reshape(H // 2, NV, 16, 128)
    xp = x5.reshape(H // 2, 2, NV, 8, 128)
    w2t = jnp.transpose(w2)

    kern = functools.partial(_kernel, H=H, C=C, E=E, W=W)
    hbm = pl.BlockSpec(memory_space=pl.ANY)
    out = pl.pallas_call(
        kern,
        in_specs=[hbm] * 7,
        out_specs=hbm,
        out_shape=jax.ShapeDtypeStruct((H // 2, NV, 16, 128), jnp.bfloat16),
        scratch_shapes=[
            pltpu.VMEM((NB * (TH - len(RC)) - GLESS, E // 2, W), u32),
            pltpu.VMEM((2, NP, NV, 16, 128), bf16),
            pltpu.VMEM((NR, 2, NV * 8, 128), u32),
            pltpu.VMEM((NR, 2, C // 2, W), u32),
            pltpu.VMEM((NV * 8, 128), u32),
            pltpu.VMEM((E, 128), f32),
            pltpu.VMEM((E // 2, C), u32),
            pltpu.VMEM((64, E), u32),
            pltpu.VMEM((64, E), u32),
            pltpu.VMEM((C, 128), f32),
            pltpu.VMEM((NG, 8, 128), u32),
            pltpu.VMEM((8, 512), f32),
            pltpu.VMEM((32, 128), f32),
            pltpu.SMEM((1,), jnp.int32),
            pltpu.SemaphoreType.DMA((2, 2)),
            pltpu.SemaphoreType.DMA((4,)),
            pltpu.SemaphoreType.DMA((4,)),
            pltpu.SemaphoreType.DMA((5,)),
        ],
        compiler_params=pltpu.CompilerParams(
            vmem_limit_bytes=128 * 1024 * 1024,
            disable_bounds_checks=True,
        ),
        name="convnext_block",
    )(xp, xn, dw, w1, w2t, grn_gamma, grn_beta)
    out = jnp.transpose(out.reshape(H, NG, NT, 8, 128), (0, 1, 3, 2, 4)).reshape(H, C, W)
    return jnp.transpose(out, (0, 2, 1))[None]
```

```python
import functools
import math

import jax
import jax.numpy as jnp
import jax.experimental.pallas as pl
import jax.experimental.pallas.tpu as pltpu

_K0 = math.sqrt(2.0 / math.pi)
_K1 = 0.044715 * _K0
_ALPHA = _K1 ** (1.0 / 3.0)
_KP = _K0 / _ALPHA
_GS = 2.0 * _ALPHA

f32 = jnp.float32
bf16 = jnp.bfloat16
u32 = jnp.uint32

NP = 8
NR = 4
TH = 8
RC = (1, 2, 3)
CH = 64
CH2 = 128
P2 = 'r0120,r1001,x000,r0200,r0100,y000,r0310,a0000,z000,b0000,c0000'
RORD = [5,6,7,0,4]
PG = 3
LDIST = 2
CSPLIT = 0
SKIP1 = 0
OPQ = 0
DMAEND = 1
GLESS = 0
N2 = 64
DIST = [4]*12
DIST0 = [0,0]+[4]*8+[8,8]
DISTL = [8,8]+[4]*8+[0,0]


def _tree_sum(vs):
    vs = list(vs)
    while len(vs) > 1:
        nxt = [vs[i] + vs[i + 1] for i in range(0, len(vs) - 1, 2)]
        if len(vs) % 2:
            nxt.append(vs[-1])
        vs = nxt
    return vs[0]


def _sub_allreduce(s):
    s = s + pltpu.roll(s, 4, 0)
    s = s + pltpu.roll(s, 2, 0)
    s = s + pltpu.roll(s, 1, 0)
    return s


def _layernorm_tile(o, C, log2_scale):
    m = _sub_allreduce(_tree_sum(o)) * (1.0 / C)
    d = [t - m for t in o]
    v = _sub_allreduce(_tree_sum([t * t for t in d]))
    r = jnp.exp2(jnp.log(v + C * 1e-5) * (-0.5 * math.log2(math.e)) + log2_scale)
    return jnp.concatenate([t * r for t in d], axis=0).astype(bf16)


def _gelu2(h):
    return h * (1.0 + jnp.tanh(h * (h * h + _KP)))


def _kernel(xp_hbm, x_hbm, dw_hbm, w1_hbm, w2t_hbm, gam_hbm, bet_hbm,
            o_hbm,
            g_s, xc_s, lr_s, y_s, cl_s, acc_s, w1t_s, w2s_s, w2f_s, bias_s, l1_s, gb_s, dwr_s, z_s,
            sem_c, sem_x, sem_o, sem_p,
            *, H, C, E, W):
    NB1 = H // (2 * NP)
    NB = H // TH
    NG = C // 8
    NT = W // 128
    NS = NG * NT // 2
    NV = NG * NT
    NCH = E // CH
    res_rows = [r for r in range(TH) if r not in RC]
    NRES = len(res_rows)
    ln_scale = math.log2(_ALPHA * math.sqrt(C))

    g_b = g_s.bitcast(bf16)
    y_b = y_s.bitcast(bf16)
    xu = xc_s.bitcast(u32)
    lane = jax.lax.broadcasted_iota(jnp.int32, (8, 128), 1)
    zero_u = jnp.zeros((8, 128), u32)
    zero_f = jnp.zeros((8, 128), f32)

    def wtap_idx(t):
        return (2 + t // 8, (t % 8) // 4)

    def build_taps():
        rows = jax.lax.broadcasted_iota(jnp.int32, (C, 128), 0)
        cols = jax.lax.broadcasted_iota(jnp.int32, (C, 128), 1)
        for t in range(9):
            col = jnp.sum(jnp.where(rows == cols, dwr_s[t:t + 1, :], 0.0), axis=1, keepdims=True)
            a, b = wtap_idx(t)
            lr_s[a, b, (t % 4) * C:(t % 4 + 1) * C, :] = pltpu.bitcast(
                jnp.broadcast_to(col, (C, 128)), u32)

    def wtap(i, j, cg):
        t = i * 3 + j
        lo = (t % 4) * C + cg * 8
        a, b = wtap_idx(t)
        return pltpu.bitcast(lr_s[a, b, lo:lo + 8, :], f32)

    pend = []

    def linked(u):
        due = [v for (n, v) in pend if n <= 1]
        pend[:] = [(n - 1, v) for (n, v) in pend if n > 1]
        if not due:
            return u
        dep = due[0]
        for v in due[1:]:
            dep = dep | v
        dep = dep & jnp.full((8, 128), z_s[0], jnp.int32).astype(u32)
        if u.shape[1] <= 128:
            dep = dep[:, 0:u.shape[1]]
        else:
            dep = jnp.concatenate([dep, jnp.zeros((8, u.shape[1] - 128), u32)], axis=1)
        return jnp.concatenate([u[0:8] | dep, u[8:]], axis=0)

    def mm1_raw(y, c, ch):
        lhs = pltpu.bitcast(linked(w1t_s[c * ch // 2:(c + 1) * ch // 2, :]), bf16)
        return jnp.dot(lhs, y, preferred_element_type=f32)

    def gelu_acc(h, c, gidx):
        g = _gelu2(h)
        g2 = g * g
        acc_s[c * CH:(c + 1) * CH, :] += _tree_sum(
            [g2[:, k * 128:(k + 1) * 128] for k in range(NT)])
        if gidx is not None:
            g_b.at[gidx][c * CH:(c + 1) * CH, :] = g.astype(bf16)

    def gindex(blk, r):
        if r % TH not in res_rows:
            return None
        b = blk * (2 * NP // TH) + r // TH
        if r < 0:
            b = jnp.maximum(b, 0)
        return b * NRES + res_rows.index(r % TH)

    def c_copies(blk, slot):
        return [
            pltpu.make_async_copy(xp_hbm.at[pl.ds(blk * NP - 1, NP), 1],
                                  xc_s.at[slot, :, :, pl.ds(0, 8), :], sem_c.at[slot, 0]),
            pltpu.make_async_copy(xp_hbm.at[pl.ds(blk * NP, NP), 0],
                                  xc_s.at[slot, :, :, pl.ds(8, 8), :], sem_c.at[slot, 1]),
        ]

    def last_copy(slot):
        return pltpu.make_async_copy(xp_hbm.at[NB1 * NP - 1, 1],
                                     xc_s.at[slot, 0, :, pl.ds(0, 8), :], sem_c.at[slot, 0])

    def setup(dw_ref, w1_ref, w2t_ref, gam_ref, bet_ref):
        bufs = (dw_ref, w1_ref, w2t_ref, gam_ref, bet_ref)
        cps = [pltpu.make_async_copy(src, dst, sem_p.at[n]) for n, (src, dst) in
               enumerate(zip((dw_hbm, w1_hbm, w2t_hbm, gam_hbm, bet_hbm), bufs))]
        for c in cps:
            c.start()
        pltpu.make_async_copy(xp_hbm.at[pl.ds(0, NP), 0],
                              xc_s.at[0, :, :, pl.ds(8, 8), :], sem_c.at[0, 1]).start()
        pltpu.make_async_copy(xp_hbm.at[pl.ds(0, NP - 1), 1],
                              xc_s.at[0, pl.ds(1, NP - 1), :, pl.ds(0, 8), :], sem_c.at[0, 0]).start()
        xc_s[1, 0, :, pl.ds(0, 8), :] = jnp.zeros((NV, 8, 128), bf16)
        pltpu.make_async_copy(xc_s.at[1, 0, :, pl.ds(0, 8), :],
                              xc_s.at[0, 0, :, pl.ds(0, 8), :], sem_c.at[0, 0]).start()
        for c in cps:
            c.wait()

        for n in range(4):
            z_s[n] = 0
        acc_s[...] = jnp.zeros(acc_s.shape, f32)
        cl_s[...] = jnp.zeros(cl_s.shape, u32)
        y_s[...] = jnp.zeros(y_s.shape, u32)
        gb_s[...] = jnp.zeros(gb_s.shape, f32)
        dwr_s[...] = jnp.zeros(dwr_s.shape, f32)
        gb_s[0:1, 0:E] = gam_ref[...].astype(f32).reshape(1, E)
        gb_s[1:2, 0:E] = bet_ref[...].astype(f32).reshape(1, E)
        w2f_s[0:C // 2, :] = pltpu.bitcast(w2t_ref[...], u32)
        w1t_s[...] = pltpu.bitcast(jnp.transpose(w1_ref[...].astype(f32)).astype(bf16), u32)
        for i in range(3):
            for j in range(3):
                dwr_s[i * 3 + j:i * 3 + j + 1, 0:C] = dw_ref[i, j:j + 1, :].astype(f32)
        build_taps()
        r16 = jax.lax.broadcasted_iota(jnp.int32, (16, 128), 0)
        c16 = jax.lax.broadcasted_iota(jnp.int32, (16, 128), 1)
        kv = c16 // 16
        kb = c16 % 16
        k_row = 2 * (kv // 3) + kb // 8 - r16 // 8
        k_j = kv % 3
        for cg in range(NG):
            l1 = jnp.zeros((16, 128), f32)
            for i in range(3):
                for j in range(3):
                    w8 = wtap(i, j, cg)
                    hit = (kb % 8 == r16 % 8) & (k_row == i) & (k_j == j) & (kv < 6)
                    l1 = jnp.where(hit, jnp.concatenate([w8, w8], axis=0), l1)
            l1_s[cg] = pltpu.bitcast(l1.astype(bf16), u32)
        lr_s[NR - 1] = jnp.zeros(lr_s.shape[1:], u32)

    pl.run_scoped(
        setup,
        pltpu.VMEM((3, 3, C), bf16),
        pltpu.VMEM((C, E), bf16),
        pltpu.VMEM((C, E), bf16),
        pltpu.VMEM((E,), bf16),
        pltpu.VMEM((E,), bf16),
    )

    def a1(slot, q):
        for cg in range(NG):
            t = [xu[slot, q, cg * NT + k] for k in range(NT)]
            for k in range(NT):
                lo = (cg * NT + k) * 8
                if q == NP - 1:
                    cl_s[lo:lo + 8, :] = t[k]
                lsrc = t[k - 1] if k > 0 else zero_u
                rsrc = t[k + 1] if k < NT - 1 else zero_u
                lr_s[q % NR, 0, lo:lo + 8, :] = pltpu.roll(jnp.where(lane == 127, lsrc, t[k]), 1, 1)
                lr_s[q % NR, 1, lo:lo + 8, :] = pltpu.roll(jnp.where(lane == 0, rsrc, t[k]), 127, 1)

    def conv_pair_dot(slot, j, cg, k):
        n = cg * NT + k
        parts = []
        for q in (j, j + 1):
            c = xu[slot, q, n] if q >= 0 else cl_s[8 * n:8 * n + 8, :]
            parts += [lr_s[q % NR, 0, 8 * n:8 * n + 8, :], c, lr_s[q % NR, 1, 8 * n:8 * n + 8, :]]
        wt = pltpu.bitcast(jnp.concatenate(parts, axis=0), bf16)
        lhs = pltpu.bitcast(l1_s[cg, :, 0:96], bf16)
        return jnp.dot(lhs, wt, preferred_element_type=f32)

    def b_and_c(slot, j, scale, yslot, gidx, dist):
        order = [(k, cg) for k in range(NT) for cg in range(NG)]
        o = {}
        pos = 0
        for n in range(2 * NCH):
            gelu_acc(mm1_raw(y_b[yslot, n // NCH], n % NCH, CH), n % NCH, gidx[n // NCH])
            for (k, cg) in order[pos:pos + dist[n]]:
                o[cg] = conv_pair_dot(slot, j, cg, k)
                if cg == NG - 1:
                    for hh in range(2):
                        yt = _layernorm_tile([o[q][8 * hh:8 * hh + 8] for q in range(NG)], C, scale)
                        y_b.at[j % NR, hh][:, k * 128:(k + 1) * 128] = yt
            pos += dist[n]

    def p1_body(i, carry):
        slot = i & 1
        for c in c_copies(1, slot):
            c.wait()

        @pl.when(i + 1 < NB1)
        def _():
            for c in c_copies(i + 1, 1 - slot):
                c.start()

        @pl.when(i + 1 == NB1)
        def _():
            last_copy(1 - slot).start()

        for j in range(-1, NP - 1):
            scale = jnp.where(i > 0, ln_scale, -1000.0) if j == -1 else ln_scale
            a1(slot, j + 1)
            jc = j - 2
            b_and_c(slot, j, scale, jc % NR, [gindex(i, 2 * jc), gindex(i, 2 * jc + 1)],
                    DIST0 if j == -1 else (DISTL if j == NP - 2 else DIST))
        return carry

    if not SKIP1:
        jax.lax.fori_loop(0, NB1, p1_body, 0)

    def xslot(s):
        return xc_s.at[s >> 1, pl.ds((s & 1) * (TH // 2), TH // 2)]

    def x_copy(blk, s):
        return pltpu.make_async_copy(x_hbm.at[pl.ds(blk * (TH // 2), TH // 2)], xslot(s), sem_x.at[s])

    def o_copy(blk, s):
        return pltpu.make_async_copy(xslot(s), o_hbm.at[pl.ds(blk * (TH // 2), TH // 2)], sem_o.at[s])

    dslot = NB1 % 2
    S0 = 2 * (1 - dslot)
    last_copy(dslot).wait()
    x_copy(0, S0).start()
    x_copy(1, S0 + 1).start()
    xc_s[dslot, 0, :, pl.ds(8, 8), :] = jnp.zeros((NV, 8, 128), bf16)
    if not SKIP1:
        a1(dslot, 0)
        b_and_c(dslot, -1, ln_scale, (-3) % NR, [gindex(NB1, -6), gindex(NB1, -5)], DIST0)
    for jc in (-2, -1) if not SKIP1 else (-1,):
        for n in range(2 * NCH):
            gelu_acc(mm1_raw(y_b[jc % NR, n // NCH], n % NCH, CH), n % NCH,
                     gindex(NB1, 2 * jc + n // NCH))

    ssq = jnp.sum(jnp.transpose(acc_s[...]), axis=0, keepdims=True)
    gx = jnp.sqrt(ssq * (1.0 / (_GS * _GS)) + 1e-6)
    nx = gx / (jnp.sum(gx, axis=1, keepdims=True) * (1.0 / E) + 1e-6)
    sc = (gb_s[0:1, 0:E] * nx + 1.0) * (1.0 / _GS)
    w2 = pltpu.bitcast(w2f_s[0:C // 2, :], bf16).astype(f32)
    w2s_s[0:C // 2, :] = pltpu.bitcast((w2 * sc).astype(bf16), u32)
    b = jnp.sum(w2 * gb_s[1:2, 0:E], axis=1, keepdims=True)
    bias_s[...] = jnp.broadcast_to(b, (C, 128))
    build_taps()
    if DMAEND:
        x_copy(2, (S0 + 2) & 3).start()

    def pass2(gt_s):
        gt_b = gt_s.bitcast(bf16)

        def o_idx(n, k, cg):
            m = (n * NT + k) * NG + cg
            return (m // (2 * NV), (m // NV) % 2, pl.ds((m % NV) * 8, 8), slice(None))

        def p2_body(i, carry):
            s = (i + S0) & 3
            sa, sb = s >> 1, (s & 1) * (TH // 2)
            x_copy(0, s).wait()

            if not DMAEND:
                @pl.when(i >= 2)
                def _():
                    o_copy(0, (s + 2) & 3).wait()

                @pl.when(i + 2 < NB)
                def _():
                    x_copy(i + 2, (s + 2) & 3).start()

            def xrow(r, slab, tag=None):
                if tag is not None and OPQ == 2:
                    u = xu[sa, sb + z_s[tag] + r // 2, (r % 2) * NS + slab]
                else:
                    u = xu[sa, sb + r // 2, (r % 2) * NS + slab]
                if tag is not None and OPQ == 1:
                    u = u | jnp.full((8, 128), z_s[tag], jnp.int32).astype(u32)
                v = pltpu.bitcast(u, bf16).astype(f32)
                return [v[0:8], v[8:16]]

            def conv_piece(n, cgs):
                outs = []
                for cg in cgs:
                    rows_ = [xrow(r, 2 * cg, 1 + n) + xrow(r, 2 * cg + 1, 1 + n) for r in range(RC[n] - 1, RC[n] + 2)]
                    w = [[wtap(ii, j, cg) for j in range(3)] for ii in range(3)]
                    t = [[rows_[0][k] * w[0][j] + rows_[1][k] * w[1][j] + rows_[2][k] * w[2][j]
                          for k in range(NT)] for j in range(3)]
                    for k in range(NT):
                        lsrc = t[0][k - 1] if k > 0 else zero_f
                        rsrc = t[2][k + 1] if k < NT - 1 else zero_f
                        left = pltpu.roll(jnp.where(lane == 127, lsrc, t[0][k]), 1, 1)
                        right = pltpu.roll(jnp.where(lane == 0, rsrc, t[2][k]), 127, 1)
                        ov = pltpu.bitcast(t[1][k] + left + right, u32)
                        lr_s[o_idx(n, k, cg)] = ov
                        outs.append(ov)
                dep = outs[0]
                for v in outs[1:]:
                    dep = dep | v
                pend.append((LDIST, dep))

            done = [False] * len(RC)

            def pieces():
                for n in range(len(RC)):
                    for c0 in range(0, NG, PG):
                        conv_piece(n, range(c0, c0 + PG))
                        if c0 + PG == NG:
                            done[n] = True
                            for k in range(NT):
                                o = [pltpu.bitcast(lr_s[o_idx(n, k, cg)], f32) for cg in range(NG)]
                                y_b.at[n // 2, n % 2][:, k * 128:(k + 1) * 128] = _layernorm_tile(
                                    o, C, ln_scale)
                        yield

            def stage_d(r, g, gen, per):
                p = []
                full = sum(per[:NT - 1]) == 0
                if full:
                    lhs = pltpu.bitcast(linked(w2s_s[0:C // 2, :]), bf16)
                    pf = jnp.dot(lhs, g, preferred_element_type=f32)
                for k in range(NT):
                    if full:
                        p.append(pf[:, k * 128:(k + 1) * 128])
                    else:
                        lhs = pltpu.bitcast(linked(w2s_s[0:C // 2, :]), bf16)
                        p.append(jnp.dot(lhs, g[:, k * 128:(k + 1) * 128], preferred_element_type=f32))
                    for _ in range(per[k]):
                        next(gen)
                assert all(done[n] for n in range(len(RC)) if abs(RC[n] - r) <= 1)
                for pp in range(NT // 2):
                    for cg in range(NG):
                        b8 = bias_s[cg * 8:cg * 8 + 8, :]
                        slab = 2 * cg + pp
                        xr = xrow(r, slab)
                        v = [xr[h] + (p[2 * pp + h][cg * 8:cg * 8 + 8] + b8) for h in range(2)]
                        xc_s[sa, sb + r // 2, (r % 2) * NS + slab] = jnp.concatenate(
                            v, axis=0).astype(bf16)

            pend.clear()
            res = list(RORD)
            gen = pieces()
            for tok in P2.split(','):
                op = tok[0]
                per = [int(c) for c in tok[1:]] + [0] * 8
                if op == 'r':
                    r = res.pop(0)
                    stage_d(r, g_b[i * NRES + res_rows.index(r)], gen, per)
                elif op in 'xyz':
                    n = 'xyz'.index(op)
                    ch = CH2 if (sum(per) or CSPLIT) else E
                    for c in range(E // ch):
                        gt_b.at[n][c * ch:(c + 1) * ch, :] = _gelu2(
                            mm1_raw(y_b[n // 2, n % 2], c, ch)).astype(bf16)
                        for _ in range(per[c]):
                            next(gen)
                else:
                    n = 'abc'.index(op)
                    stage_d(RC[n], gt_b[n], gen, per)
            assert not res and next(gen, 'done') == 'done'
            pend.clear()
            o_copy(i, s).start()
            if DMAEND:
                @pl.when(i >= 1)
                def _():
                    o_copy(0, (s + 3) & 3).wait()

                @pl.when(i + 3 < NB)
                def _():
                    x_copy(i + 3, (s + 3) & 3).start()
            return carry

        jax.lax.fori_loop(0, N2, p2_body, 0)
        if not DMAEND:
            o_copy(0, (N2 - 2 + S0) & 3).wait()
        o_copy(0, (N2 - 1 + S0) & 3).wait()
        if N2 < NB:
            x_copy(0, (N2 + S0) & 3).wait()
        if N2 + 1 < NB:
            x_copy(0, (N2 + 1 + S0) & 3).wait()
        if N2 + 2 < NB and DMAEND:
            x_copy(0, (N2 + 2 + S0) & 3).wait()

    pl.run_scoped(pass2, pltpu.VMEM((len(RC), E // 2, W), u32))


@jax.jit
def pallas_standalone__modern_conv_block_convnext_v2__vision_kernel(
    x: jax.Array,
    dw: jax.Array,
    w1: jax.Array,
    w2: jax.Array,
    grn_gamma: jax.Array,
    grn_beta: jax.Array,
):
    B, H, W, C = x.shape
    E = w1.shape[1]
    assert B == 1
    NB = H // TH
    NG = C // 8
    NT = W // 128
    NV = NG * NT
    x5 = jnp.transpose(x[0], (0, 2, 1)).reshape(H, NG, 8, NT, 128)
    x5 = jnp.transpose(x5, (0, 1, 3, 2, 4))
    xn = x5.reshape(H // 2, NV, 16, 128)
    xp = x5.reshape(H // 2, 2, NV, 8, 128)
    w2t = jnp.transpose(w2)

    kern = functools.partial(_kernel, H=H, C=C, E=E, W=W)
    hbm = pl.BlockSpec(memory_space=pl.ANY)
    out = pl.pallas_call(
        kern,
        in_specs=[hbm] * 7,
        out_specs=hbm,
        out_shape=jax.ShapeDtypeStruct((H // 2, NV, 16, 128), jnp.bfloat16),
        scratch_shapes=[
            pltpu.VMEM((NB * (TH - len(RC)) - GLESS, E // 2, W), u32),
            pltpu.VMEM((2, NP, NV, 16, 128), bf16),
            pltpu.VMEM((NR, 2, NV * 8, 128), u32),
            pltpu.VMEM((NR, 2, C // 2, W), u32),
            pltpu.VMEM((NV * 8, 128), u32),
            pltpu.VMEM((E, 128), f32),
            pltpu.VMEM((E // 2, C), u32),
            pltpu.VMEM((64, E), u32),
            pltpu.VMEM((64, E), u32),
            pltpu.VMEM((C, 128), f32),
            pltpu.VMEM((NG, 8, 128), u32),
            pltpu.VMEM((8, 512), f32),
            pltpu.VMEM((32, 128), f32),
            pltpu.SMEM((4,), jnp.int32),
            pltpu.SemaphoreType.DMA((2, 2)),
            pltpu.SemaphoreType.DMA((4,)),
            pltpu.SemaphoreType.DMA((4,)),
            pltpu.SemaphoreType.DMA((5,)),
        ],
        compiler_params=pltpu.CompilerParams(
            vmem_limit_bytes=128 * 1024 * 1024,
            disable_bounds_checks=True,
        ),
        name="convnext_block",
    )(xp, xn, dw, w1, w2t, grn_gamma, grn_beta)
    out = jnp.transpose(out.reshape(H, NG, NT, 8, 128), (0, 1, 3, 2, 4)).reshape(H, C, W)
    return jnp.transpose(out, (0, 2, 1))[None]
```

```python
import functools
import math

import jax
import jax.numpy as jnp
import jax.experimental.pallas as pl
import jax.experimental.pallas.tpu as pltpu

_K0 = math.sqrt(2.0 / math.pi)
_K1 = 0.044715 * _K0
_ALPHA = _K1 ** (1.0 / 3.0)
_KP = _K0 / _ALPHA
_GS = 2.0 * _ALPHA

f32 = jnp.float32
bf16 = jnp.bfloat16
u32 = jnp.uint32

NP = 8
NR = 4
TH = 8
RC = (1, 2, 3)
CH = 64
CH2 = 128
P2 = 'r0120,r1001,x000,r0200,r0100,y000,r0310,a0000,z000,b0000,c0000'
RORD = [5,6,7,0,4]
PG = 3
LDIST = 2
CSPLIT = 0
SKIP1 = 0
OPQ = 0
DMAEND = 1
SH = 1
ND = 1
HL = 3
LSTEP = 1
LNL = 0
LNS = 0
GL = 0
GS = 32
GLESS = 0
N2 = 64
DIST = [4]*12
DIST0 = [0,0]+[4]*8+[8,8]
DISTL = [8,8]+[4]*8+[0,0]


def _tree_sum(vs):
    vs = list(vs)
    while len(vs) > 1:
        nxt = [vs[i] + vs[i + 1] for i in range(0, len(vs) - 1, 2)]
        if len(vs) % 2:
            nxt.append(vs[-1])
        vs = nxt
    return vs[0]


def _sub_allreduce(s):
    s = s + pltpu.roll(s, 4, 0)
    s = s + pltpu.roll(s, 2, 0)
    s = s + pltpu.roll(s, 1, 0)
    return s


def _layernorm_tile(o, C, log2_scale, out=None):
    m = _sub_allreduce(_tree_sum(o)) * (1.0 / C)
    d = [t - m for t in o]
    v = _sub_allreduce(_tree_sum([t * t for t in d]))
    r = jnp.exp2(jnp.log(v + C * 1e-5) * (-0.5 * math.log2(math.e)) + log2_scale)
    y = [t * r for t in d]
    if out is not None:
        out.extend(y)
    return jnp.concatenate(y, axis=0).astype(bf16)


def _gelu2(h):
    return h * (1.0 + jnp.tanh(h * (h * h + _KP)))


def _kernel(xp_hbm, x_hbm, dw_hbm, w1_hbm, w2t_hbm, gam_hbm, bet_hbm,
            o_hbm,
            g_s, xc_s, lr_s, y_s, cl_s, od_s, acc_s, w1t_s, w2s_s, w2f_s, bias_s, l1_s, gb_s, dwr_s, z_s,
            sem_c, sem_x, sem_o, sem_p,
            *, H, C, E, W):
    NB1 = H // (2 * NP)
    NB = H // TH
    NG = C // 8
    NT = W // 128
    NS = NG * NT // 2
    NV = NG * NT
    NCH = E // CH
    res_rows = [r for r in range(TH) if r not in RC]
    NRES = len(res_rows)
    ln_scale = math.log2(_ALPHA * math.sqrt(C))

    g_b = g_s.bitcast(bf16)
    y_b = y_s.bitcast(bf16)
    xu = xc_s.bitcast(u32)
    lane = jax.lax.broadcasted_iota(jnp.int32, (8, 128), 1)
    zero_u = jnp.zeros((8, 128), u32)
    zero_f = jnp.zeros((8, 128), f32)

    def wtap_idx(t):
        return (2 + t // 8, (t % 8) // 4)

    def build_taps():
        rows = jax.lax.broadcasted_iota(jnp.int32, (C, 128), 0)
        cols = jax.lax.broadcasted_iota(jnp.int32, (C, 128), 1)
        for t in range(9):
            col = jnp.sum(jnp.where(rows == cols, dwr_s[t:t + 1, :], 0.0), axis=1, keepdims=True)
            a, b = wtap_idx(t)
            lr_s[a, b, (t % 4) * C:(t % 4 + 1) * C, :] = pltpu.bitcast(
                jnp.broadcast_to(col, (C, 128)), u32)

    def wtap(i, j, cg):
        t = i * 3 + j
        lo = (t % 4) * C + cg * 8
        a, b = wtap_idx(t)
        return pltpu.bitcast(lr_s[a, b, lo:lo + 8, :], f32)

    pend = []

    def linked(u):
        due = [v for (n, v) in pend if n <= 1]
        pend[:] = [(n - 1, v) for (n, v) in pend if n > 1]
        if not due:
            return u
        dep = due[0]
        for v in due[1:]:
            dep = dep | v
        dep = dep & jnp.full((8, 128), z_s[0], jnp.int32).astype(u32)
        if u.shape[1] <= 128:
            dep = dep[:, 0:u.shape[1]]
        else:
            dep = jnp.concatenate([dep, jnp.zeros((8, u.shape[1] - 128), u32)], axis=1)
        return jnp.concatenate([u[0:8] | dep, u[8:]], axis=0)

    def mm1_raw(y, c, ch):
        lhs = pltpu.bitcast(linked(w1t_s[c * ch // 2:(c + 1) * ch // 2, :]), bf16)
        return jnp.dot(lhs, y, preferred_element_type=f32)

    def gelu_acc(h, c, gidx):
        g = _gelu2(h)
        g2 = g * g
        acc_s[c * CH:(c + 1) * CH, :] += _tree_sum(
            [g2[:, k * 128:(k + 1) * 128] for k in range(NT)])
        if gidx is not None:
            g_b.at[gidx][c * CH:(c + 1) * CH, :] = g.astype(bf16)

    def gindex(blk, r):
        if r % TH not in res_rows:
            return None
        b = blk * (2 * NP // TH) + r // TH
        if r < 0:
            b = jnp.maximum(b, 0)
        return b * NRES + res_rows.index(r % TH)

    def c_copies(blk, slot):
        return [
            pltpu.make_async_copy(xp_hbm.at[pl.ds(blk * NP - 1, NP), 1],
                                  xc_s.at[slot, :, :, pl.ds(0, 8), :], sem_c.at[slot, 0]),
            pltpu.make_async_copy(xp_hbm.at[pl.ds(blk * NP, NP), 0],
                                  xc_s.at[slot, :, :, pl.ds(8, 8), :], sem_c.at[slot, 1]),
        ]

    def last_copy(slot):
        return pltpu.make_async_copy(xp_hbm.at[NB1 * NP - 1, 1],
                                     xc_s.at[slot, 0, :, pl.ds(0, 8), :], sem_c.at[slot, 0])

    def setup(dw_ref, w1_ref, w2t_ref, gam_ref, bet_ref):
        bufs = (dw_ref, w1_ref, w2t_ref, gam_ref, bet_ref)
        cps = [pltpu.make_async_copy(src, dst, sem_p.at[n]) for n, (src, dst) in
               enumerate(zip((dw_hbm, w1_hbm, w2t_hbm, gam_hbm, bet_hbm), bufs))]
        for c in cps:
            c.start()
        pltpu.make_async_copy(xp_hbm.at[pl.ds(0, NP), 0],
                              xc_s.at[0, :, :, pl.ds(8, 8), :], sem_c.at[0, 1]).start()
        pltpu.make_async_copy(xp_hbm.at[pl.ds(0, NP - 1), 1],
                              xc_s.at[0, pl.ds(1, NP - 1), :, pl.ds(0, 8), :], sem_c.at[0, 0]).start()
        xc_s[1, 0, :, pl.ds(0, 8), :] = jnp.zeros((NV, 8, 128), bf16)
        pltpu.make_async_copy(xc_s.at[1, 0, :, pl.ds(0, 8), :],
                              xc_s.at[0, 0, :, pl.ds(0, 8), :], sem_c.at[0, 0]).start()
        for c in cps:
            c.wait()

        for n in range(4):
            z_s[n] = 0
        acc_s[...] = jnp.zeros(acc_s.shape, f32)
        cl_s[...] = jnp.zeros(cl_s.shape, u32)
        od_s[...] = jnp.zeros(od_s.shape, f32)
        y_s[...] = jnp.zeros(y_s.shape, u32)
        gb_s[...] = jnp.zeros(gb_s.shape, f32)
        dwr_s[...] = jnp.zeros(dwr_s.shape, f32)
        gb_s[0:1, 0:E] = gam_ref[...].astype(f32).reshape(1, E)
        gb_s[1:2, 0:E] = bet_ref[...].astype(f32).reshape(1, E)
        w2f_s[0:C // 2, :] = pltpu.bitcast(w2t_ref[...], u32)
        w1t_s[...] = pltpu.bitcast(jnp.transpose(w1_ref[...].astype(f32)).astype(bf16), u32)
        for i in range(3):
            for j in range(3):
                dwr_s[i * 3 + j:i * 3 + j + 1, 0:C] = dw_ref[i, j:j + 1, :].astype(f32)
        build_taps()
        r16 = jax.lax.broadcasted_iota(jnp.int32, (16, 128), 0)
        c16 = jax.lax.broadcasted_iota(jnp.int32, (16, 128), 1)
        kv = c16 // 16
        kb = c16 % 16
        k_row = 2 * (kv // 3) + kb // 8 - r16 // 8
        k_j = kv % 3
        for cg in range(NG):
            l1 = jnp.zeros((16, 128), f32)
            for i in range(3):
                for j in range(3):
                    w8 = wtap(i, j, cg)
                    hit = (kb % 8 == r16 % 8) & (k_row == i) & (k_j == j) & (kv < 6)
                    l1 = jnp.where(hit, jnp.concatenate([w8, w8], axis=0), l1)
            l1_s[cg] = pltpu.bitcast(l1.astype(bf16), u32)
        lr_s[NR - 1] = jnp.zeros(lr_s.shape[1:], u32)
        lr_s[NR - 2] = jnp.zeros(lr_s.shape[1:], u32)

    pl.run_scoped(
        setup,
        pltpu.VMEM((3, 3, C), bf16),
        pltpu.VMEM((C, E), bf16),
        pltpu.VMEM((C, E), bf16),
        pltpu.VMEM((E,), bf16),
        pltpu.VMEM((E,), bf16),
    )

    def a1(slot, q):
        for cg in range(NG):
            t = [xu[slot, q, cg * NT + k] for k in range(NT)]
            for k in range(NT):
                lo = (cg * NT + k) * 8
                if q == NP - 1:
                    cl_s[lo:lo + 8, :] = t[k]
                if q == NP - 2 and k >= NT - SH:
                    l2 = (NV + cg * SH + k - (NT - SH)) * 8
                    cl_s[l2:l2 + 8, :] = t[k]
                lsrc = t[k - 1] if k > 0 else zero_u
                rsrc = t[k + 1] if k < NT - 1 else zero_u
                lr_s[q % NR, 0, lo:lo + 8, :] = pltpu.roll(jnp.where(lane == 127, lsrc, t[k]), 1, 1)
                lr_s[q % NR, 1, lo:lo + 8, :] = pltpu.roll(jnp.where(lane == 0, rsrc, t[k]), 127, 1)

    def conv_pair_dot(slot, j, cg, k):
        n = cg * NT + k
        parts = []
        for q in (j, j + 1):
            m = n if q == -1 else NV + cg * SH + k - (NT - SH)
            c = xu[slot, q, n] if q >= 0 else cl_s[8 * m:8 * m + 8, :]
            parts += [lr_s[q % NR, 0, 8 * n:8 * n + 8, :], c, lr_s[q % NR, 1, 8 * n:8 * n + 8, :]]
        wt = pltpu.bitcast(jnp.concatenate(parts, axis=0), bf16)
        lhs = pltpu.bitcast(l1_s[cg, :, 0:96], bf16)
        return jnp.dot(lhs, wt, preferred_element_type=f32)

    def ln_unit(o, j, k, scale, link):
        ys = []
        for hh in range(2):
            yt = _layernorm_tile([o[q][8 * hh:8 * hh + 8] for q in range(NG)], C, scale, ys)
            y_b.at[j % NR, hh][:, k * 128:(k + 1) * 128] = yt
        if link:
            ys = [pltpu.bitcast(v, u32) for v in ys[LSTEP - 1::LSTEP]]
            dep = ys[0]
            for v in ys[1:]:
                dep = dep | v
            pend.append((link, dep))

    def dot_stream(slot, units, first_scale, defer):
        for u, (j, k) in enumerate(units):
            if k == 0 and j + 1 >= 0:
                a1(slot, j + 1)
            o = []
            for cg in range(NG):
                o.append(conv_pair_dot(slot, j, cg, k))
                if cg == NG - 1:
                    if u >= len(units) - defer:
                        od_s[u - (len(units) - defer)] = jnp.concatenate(o, axis=0)
                    else:
                        ln_unit(o, j, k, first_scale if j == -1 else ln_scale, 0)
                if cg % 4 == 3:
                    yield

    def deferred_ln():
        for d in range(ND):
            o = [od_s[d, 16 * cg:16 * cg + 16, :] for cg in range(NG)]
            ln_unit(o, -2, NT - SH - ND + d, ln_scale, HL)

    def c_stream(blk, pairs, gen, skip):
        n_gap = 0
        for jc in pairs:
            for n in range(2 * NCH):
                gelu_acc(mm1_raw(y_b[jc % NR, n // NCH], n % NCH, CH), n % NCH,
                         gindex(blk, 2 * jc + n // NCH))
                if n_gap >= skip:
                    next(gen, None)
                n_gap += 1

    carry_units = [(-2, k) for k in range(NT - SH, NT)]

    def p1_body(i, carry):
        slot = i & 1
        for c in c_copies(1, slot):
            c.wait()

        @pl.when(i + 1 < NB1)
        def _():
            for c in c_copies(i + 1, 1 - slot):
                c.start()

        @pl.when(i + 1 == NB1)
        def _():
            last_copy(1 - slot).start()

        deferred_ln()
        units = carry_units + [(j, k) for j in range(-1, NP - 1) for k in range(NT)]
        units = units[:NP * NT]
        gen = dot_stream(slot, units, jnp.where(i > 0, ln_scale, -1000.0), ND)
        c_stream(i, range(-3, NP - 3), gen, 0)
        assert next(gen, 'done') == 'done'
        return carry

    if not SKIP1:
        jax.lax.fori_loop(0, NB1, p1_body, 0)

    def xslot(s):
        return xc_s.at[s >> 1, pl.ds((s & 1) * (TH // 2), TH // 2)]

    def x_copy(blk, s):
        return pltpu.make_async_copy(x_hbm.at[pl.ds(blk * (TH // 2), TH // 2)], xslot(s), sem_x.at[s])

    def o_copy(blk, s):
        return pltpu.make_async_copy(xslot(s), o_hbm.at[pl.ds(blk * (TH // 2), TH // 2)], sem_o.at[s])

    dslot = NB1 % 2
    S0 = 2 * (1 - dslot)
    last_copy(dslot).wait()
    x_copy(0, S0).start()
    x_copy(1, S0 + 1).start()
    xc_s[dslot, 0, :, pl.ds(8, 8), :] = jnp.zeros((NV, 8, 128), bf16)
    if not SKIP1:
        deferred_ln()
        gen = dot_stream(dslot, carry_units + [(-1, k) for k in range(NT)], ln_scale, 0)
        c_stream(NB1, range(-3, 0), gen, 0)
        assert next(gen, 'done') == 'done'

    ssq = jnp.sum(jnp.transpose(acc_s[...]), axis=0, keepdims=True)
    gx = jnp.sqrt(ssq * (1.0 / (_GS * _GS)) + 1e-6)
    nx = gx / (jnp.sum(gx, axis=1, keepdims=True) * (1.0 / E) + 1e-6)
    sc = (gb_s[0:1, 0:E] * nx + 1.0) * (1.0 / _GS)
    w2 = pltpu.bitcast(w2f_s[0:C // 2, :], bf16).astype(f32)
    w2s_s[0:C // 2, :] = pltpu.bitcast((w2 * sc).astype(bf16), u32)
    b = jnp.sum(w2 * gb_s[1:2, 0:E], axis=1, keepdims=True)
    bias_s[...] = jnp.broadcast_to(b, (C, 128))
    build_taps()
    if DMAEND:
        x_copy(2, (S0 + 2) & 3).start()

    def pass2(gt_s):
        gt_b = gt_s.bitcast(bf16)

        def o_idx(n, k, cg):
            m = (n * NT + k) * NG + cg
            return (m // (2 * NV), (m // NV) % 2, pl.ds((m % NV) * 8, 8), slice(None))

        def p2_body(i, carry):
            s = (i + S0) & 3
            sa, sb = s >> 1, (s & 1) * (TH // 2)
            x_copy(0, s).wait()

            if not DMAEND:
                @pl.when(i >= 2)
                def _():
                    o_copy(0, (s + 2) & 3).wait()

                @pl.when(i + 2 < NB)
                def _():
                    x_copy(i + 2, (s + 2) & 3).start()

            def xrow(r, slab, tag=None):
                if tag is not None and OPQ == 2:
                    u = xu[sa, sb + z_s[tag] + r // 2, (r % 2) * NS + slab]
                else:
                    u = xu[sa, sb + r // 2, (r % 2) * NS + slab]
                if tag is not None and OPQ == 1:
                    u = u | jnp.full((8, 128), z_s[tag], jnp.int32).astype(u32)
                v = pltpu.bitcast(u, bf16).astype(f32)
                return [v[0:8], v[8:16]]

            def conv_piece(n, cgs):
                outs = []
                for cg in cgs:
                    rows_ = [xrow(r, 2 * cg, 1 + n) + xrow(r, 2 * cg + 1, 1 + n) for r in range(RC[n] - 1, RC[n] + 2)]
                    w = [[wtap(ii, j, cg) for j in range(3)] for ii in range(3)]
                    t = [[rows_[0][k] * w[0][j] + rows_[1][k] * w[1][j] + rows_[2][k] * w[2][j]
                          for k in range(NT)] for j in range(3)]
                    for k in range(NT):
                        lsrc = t[0][k - 1] if k > 0 else zero_f
                        rsrc = t[2][k + 1] if k < NT - 1 else zero_f
                        left = pltpu.roll(jnp.where(lane == 127, lsrc, t[0][k]), 1, 1)
                        right = pltpu.roll(jnp.where(lane == 0, rsrc, t[2][k]), 127, 1)
                        ov = pltpu.bitcast(t[1][k] + left + right, u32)
                        lr_s[o_idx(n, k, cg)] = ov
                        outs.append(ov)
                dep = outs[0]
                for v in outs[1:]:
                    dep = dep | v
                pend.append((LDIST, dep))

            done = [False] * len(RC)

            def pieces():
                for n in range(len(RC)):
                    for c0 in range(0, NG, PG):
                        conv_piece(n, range(c0, c0 + PG))
                        if c0 + PG == NG:
                            done[n] = True
                            for k in range(NT):
                                o = [pltpu.bitcast(lr_s[o_idx(n, k, cg)], f32) for cg in range(NG)]
                                ys = []
                                y_b.at[n // 2, n % 2][:, k * 128:(k + 1) * 128] = _layernorm_tile(
                                    o, C, ln_scale, ys)
                                if LNL:
                                    dep = pltpu.bitcast(ys[0], u32)
                                    for v in ys[1:]:
                                        dep = dep | pltpu.bitcast(v, u32)
                                    pend.append((LNL + (k if LNS else 0), dep))
                        yield

            def stage_d(r, g, gen, per):
                p = []
                full = sum(per[:NT - 1]) == 0
                if full:
                    lhs = pltpu.bitcast(linked(w2s_s[0:C // 2, :]), bf16)
                    pf = jnp.dot(lhs, g, preferred_element_type=f32)
                for k in range(NT):
                    if full:
                        p.append(pf[:, k * 128:(k + 1) * 128])
                    else:
                        lhs = pltpu.bitcast(linked(w2s_s[0:C // 2, :]), bf16)
                        p.append(jnp.dot(lhs, g[:, k * 128:(k + 1) * 128], preferred_element_type=f32))
                    for _ in range(per[k]):
                        next(gen)
                assert all(done[n] for n in range(len(RC)) if abs(RC[n] - r) <= 1)
                for pp in range(NT // 2):
                    for cg in range(NG):
                        b8 = bias_s[cg * 8:cg * 8 + 8, :]
                        slab = 2 * cg + pp
                        xr = xrow(r, slab)
                        v = [xr[h] + (p[2 * pp + h][cg * 8:cg * 8 + 8] + b8) for h in range(2)]
                        xc_s[sa, sb + r // 2, (r % 2) * NS + slab] = jnp.concatenate(
                            v, axis=0).astype(bf16)

            pend.clear()
            res = list(RORD)
            gen = pieces()
            for tok in P2.split(','):
                op = tok[0]
                per = [int(c) for c in tok[1:]] + [0] * 8
                if op == 'r':
                    r = res.pop(0)
                    stage_d(r, g_b[i * NRES + res_rows.index(r)], gen, per)
                elif op in 'xyz':
                    n = 'xyz'.index(op)
                    ch = CH2 if (sum(per) or CSPLIT) else E
                    for c in range(E // ch):
                        gg = _gelu2(mm1_raw(y_b[n // 2, n % 2], c, ch))
                        gt_b.at[n][c * ch:(c + 1) * ch, :] = gg.astype(bf16)
                        if GL:
                            vs = [pltpu.bitcast(gg[r0:r0 + 8, W - 128:W], u32) for r0 in range(GS - 8, ch, GS)]
                            dep = vs[0]
                            for v in vs[1:]:
                                dep = dep | v
                            pend.append((GL, dep))
                        for _ in range(per[c]):
                            next(gen)
                else:
                    n = 'abc'.index(op)
                    stage_d(RC[n], gt_b[n], gen, per)
            assert not res and next(gen, 'done') == 'done'
            pend.clear()
            o_copy(i, s).start()
            if DMAEND:
                @pl.when(i >= 1)
                def _():
                    o_copy(0, (s + 3) & 3).wait()

                @pl.when(i + 3 < NB)
                def _():
                    x_copy(i + 3, (s + 3) & 3).start()
            return carry

        jax.lax.fori_loop(0, N2, p2_body, 0)
        if not DMAEND:
            o_copy(0, (N2 - 2 + S0) & 3).wait()
        o_copy(0, (N2 - 1 + S0) & 3).wait()
        if N2 < NB:
            x_copy(0, (N2 + S0) & 3).wait()
        if N2 + 1 < NB:
            x_copy(0, (N2 + 1 + S0) & 3).wait()
        if N2 + 2 < NB and DMAEND:
            x_copy(0, (N2 + 2 + S0) & 3).wait()

    pl.run_scoped(pass2, pltpu.VMEM((len(RC), E // 2, W), u32))


@jax.jit
def pallas_standalone__modern_conv_block_convnext_v2__vision_kernel(
    x: jax.Array,
    dw: jax.Array,
    w1: jax.Array,
    w2: jax.Array,
    grn_gamma: jax.Array,
    grn_beta: jax.Array,
):
    B, H, W, C = x.shape
    E = w1.shape[1]
    assert B == 1
    NB = H // TH
    NG = C // 8
    NT = W // 128
    NV = NG * NT
    x5 = jnp.transpose(x[0], (0, 2, 1)).reshape(H, NG, 8, NT, 128)
    x5 = jnp.transpose(x5, (0, 1, 3, 2, 4))
    xn = x5.reshape(H // 2, NV, 16, 128)
    xp = x5.reshape(H // 2, 2, NV, 8, 128)
    w2t = jnp.transpose(w2)

    kern = functools.partial(_kernel, H=H, C=C, E=E, W=W)
    hbm = pl.BlockSpec(memory_space=pl.ANY)
    out = pl.pallas_call(
        kern,
        in_specs=[hbm] * 7,
        out_specs=hbm,
        out_shape=jax.ShapeDtypeStruct((H // 2, NV, 16, 128), jnp.bfloat16),
        scratch_shapes=[
            pltpu.VMEM((NB * (TH - len(RC)) - GLESS, E // 2, W), u32),
            pltpu.VMEM((2, NP, NV, 16, 128), bf16),
            pltpu.VMEM((NR, 2, NV * 8, 128), u32),
            pltpu.VMEM((NR, 2, C // 2, W), u32),
            pltpu.VMEM(((NV + NG * 2) * 8, 128), u32),
            pltpu.VMEM((max(ND, 1), 2 * C, 128), f32),
            pltpu.VMEM((E, 128), f32),
            pltpu.VMEM((E // 2, C), u32),
            pltpu.VMEM((C // 2, E), u32),
            pltpu.VMEM((C // 2, E), u32),
            pltpu.VMEM((C, 128), f32),
            pltpu.VMEM((NG, 8, 128), u32),
            pltpu.VMEM((8, 512), f32),
            pltpu.VMEM((16, 128), f32),
            pltpu.SMEM((4,), jnp.int32),
            pltpu.SemaphoreType.DMA((2, 2)),
            pltpu.SemaphoreType.DMA((4,)),
            pltpu.SemaphoreType.DMA((4,)),
            pltpu.SemaphoreType.DMA((5,)),
        ],
        compiler_params=pltpu.CompilerParams(
            vmem_limit_bytes=128 * 1024 * 1024,
            disable_bounds_checks=True,
        ),
        name="convnext_block",
    )(xp, xn, dw, w1, w2t, grn_gamma, grn_beta)
    out = jnp.transpose(out.reshape(H, NG, NT, 8, 128), (0, 1, 3, 2, 4)).reshape(H, C, W)
    return jnp.transpose(out, (0, 2, 1))[None]
```

```python
import functools
import math

import jax
import jax.numpy as jnp
import jax.experimental.pallas as pl
import jax.experimental.pallas.tpu as pltpu

_K0 = math.sqrt(2.0 / math.pi)
_K1 = 0.044715 * _K0
_ALPHA = _K1 ** (1.0 / 3.0)
_KP = _K0 / _ALPHA
_GS = 2.0 * _ALPHA

f32 = jnp.float32
bf16 = jnp.bfloat16
u32 = jnp.uint32

NP = 8
NR = 4
TH = 8
RC = (1, 2, 3)
CH = 64
CH2 = 128
P2 = 'r,p,r,r,r,r,r,p,r,r,r,p,r,r,r,r,r,p,p,r,p,r,X0,p,p,r,r,p,r,X1,r,A0,X2,A1,A2'
RORD = [5,6,7,0,4]
PG = 4
LDIST = 3
CSPLIT = 0
SKIP1 = 0
OPQ = 0
DMAEND = 1
SH = 1
ND = 1
HL = 3
LSTEP = 1
LNL = 0
LNS = 0
GL = 0
GS = 32
V_SER = 0
V_G = 0
V_A = 0
GLESS = 0
N2 = 64
DIST = [4]*12
DIST0 = [0,0]+[4]*8+[8,8]
DISTL = [8,8]+[4]*8+[0,0]


def _tree_sum(vs):
    vs = list(vs)
    while len(vs) > 1:
        nxt = [vs[i] + vs[i + 1] for i in range(0, len(vs) - 1, 2)]
        if len(vs) % 2:
            nxt.append(vs[-1])
        vs = nxt
    return vs[0]


def _sub_allreduce(s):
    s = s + pltpu.roll(s, 4, 0)
    s = s + pltpu.roll(s, 2, 0)
    s = s + pltpu.roll(s, 1, 0)
    return s


def _layernorm_tile(o, C, log2_scale, out=None):
    if V_SER:
        s0 = _tree_sum(o[:8])
        s1 = _tree_sum(o[8:])
        m = _sub_allreduce(s0 + s1) * (1.0 / C)
    else:
        m = _sub_allreduce(_tree_sum(o)) * (1.0 / C)
    d = [t - m for t in o]
    v = _sub_allreduce(_tree_sum([t * t for t in d]))
    r = jnp.exp2(jnp.log(v + C * 1e-5) * (-0.5 * math.log2(math.e)) + log2_scale)
    y = [t * r for t in d]
    if out is not None:
        out.extend(y)
    return jnp.concatenate(y, axis=0).astype(bf16)


def _gelu2(h):
    if V_G == 1:
        return h + h * jnp.tanh(h * (h * h + _KP))
    return h * (1.0 + jnp.tanh(h * (h * h + _KP)))


def _kernel(xp_hbm, x_hbm, dw_hbm, w1_hbm, w2t_hbm, gam_hbm, bet_hbm,
            o_hbm,
            g_s, xc_s, lr_s, y_s, cl_s, od_s, acc_s, w1t_s, w2s_s, bias_s, l1_s, gb_s, dwr_s, z_s,
            sem_c, sem_x, sem_o, sem_p,
            *, H, C, E, W):
    NB1 = H // (2 * NP)
    NB = H // TH
    NG = C // 8
    NT = W // 128
    NS = NG * NT // 2
    NV = NG * NT
    NCH = E // CH
    res_rows = [r for r in range(TH) if r not in RC]
    NRES = len(res_rows)
    ln_scale = math.log2(_ALPHA * math.sqrt(C))

    g_b = g_s.bitcast(bf16)
    y_b = y_s.bitcast(bf16)
    xu = xc_s.bitcast(u32)
    lane = jax.lax.broadcasted_iota(jnp.int32, (8, 128), 1)
    zero_u = jnp.zeros((8, 128), u32)
    zero_f = jnp.zeros((8, 128), f32)

    def wtap_idx(t):
        return (2 + t // 8, (t % 8) // 4)

    def build_taps():
        rows = jax.lax.broadcasted_iota(jnp.int32, (C, 128), 0)
        cols = jax.lax.broadcasted_iota(jnp.int32, (C, 128), 1)
        for t in range(9):
            col = jnp.sum(jnp.where(rows == cols, dwr_s[t:t + 1, :], 0.0), axis=1, keepdims=True)
            a, b = wtap_idx(t)
            lr_s[a, b, (t % 4) * C:(t % 4 + 1) * C, :] = pltpu.bitcast(
                jnp.broadcast_to(col, (C, 128)), u32)

    def wtap(i, j, cg):
        t = i * 3 + j
        lo = (t % 4) * C + cg * 8
        a, b = wtap_idx(t)
        return pltpu.bitcast(lr_s[a, b, lo:lo + 8, :], f32)

    pend = []

    def linked(u):
        due = [v for (n, v) in pend if n <= 1]
        pend[:] = [(n - 1, v) for (n, v) in pend if n > 1]
        if not due:
            return u
        dep = due[0]
        for v in due[1:]:
            dep = dep | v
        dep = dep & jnp.full((8, 128), z_s[0], jnp.int32).astype(u32)
        if u.shape[1] <= 128:
            dep = dep[:, 0:u.shape[1]]
        else:
            dep = jnp.concatenate([dep, jnp.zeros((8, u.shape[1] - 128), u32)], axis=1)
        return jnp.concatenate([u[0:8] | dep, u[8:]], axis=0)

    def mm1_raw(y, c, ch):
        lhs = pltpu.bitcast(linked(w1t_s[c * ch // 2:(c + 1) * ch // 2, :]), bf16)
        return jnp.dot(lhs, y, preferred_element_type=f32)

    def gelu_acc(h, c, gidx):
        g = _gelu2(h)
        g2 = g * g
        if V_A == 1:
            a = acc_s[c * CH:(c + 1) * CH, :]
            for k in range(NT):
                a = a + g2[:, k * 128:(k + 1) * 128]
            acc_s[c * CH:(c + 1) * CH, :] = a
        elif V_A == 2:
            a = acc_s[c * CH:(c + 1) * CH, :]
            acc_s[c * CH:(c + 1) * CH, :] = ((a + g2[:, 0:128]) + g2[:, 128:256]) + (g2[:, 256:384] + g2[:, 384:512])
        else:
            acc_s[c * CH:(c + 1) * CH, :] += _tree_sum(
                [g2[:, k * 128:(k + 1) * 128] for k in range(NT)])
        if gidx is not None:
            g_b.at[gidx][c * CH:(c + 1) * CH, :] = g.astype(bf16)

    def gindex(blk, r):
        if r % TH not in res_rows:
            return None
        b = blk * (2 * NP // TH) + r // TH
        if r < 0:
            b = jnp.maximum(b, 0)
        return b * NRES + res_rows.index(r % TH)

    def c_copies(blk, slot):
        return [
            pltpu.make_async_copy(xp_hbm.at[pl.ds(blk * NP - 1, NP), 1],
                                  xc_s.at[slot, :, :, pl.ds(0, 8), :], sem_c.at[slot, 0]),
            pltpu.make_async_copy(xp_hbm.at[pl.ds(blk * NP, NP), 0],
                                  xc_s.at[slot, :, :, pl.ds(8, 8), :], sem_c.at[slot, 1]),
        ]

    def last_copy(slot):
        return pltpu.make_async_copy(xp_hbm.at[NB1 * NP - 1, 1],
                                     xc_s.at[slot, 0, :, pl.ds(0, 8), :], sem_c.at[slot, 0])

    def setup(dw_ref, w1_ref, w2t_ref, gam_ref, bet_ref):
        bufs = (dw_ref, w1_ref, w2t_ref, gam_ref, bet_ref)
        cps = [pltpu.make_async_copy(src, dst, sem_p.at[n]) for n, (src, dst) in
               enumerate(zip((dw_hbm, w1_hbm, w2t_hbm, gam_hbm, bet_hbm), bufs))]
        for c in cps:
            c.start()
        pltpu.make_async_copy(xp_hbm.at[pl.ds(0, NP), 0],
                              xc_s.at[0, :, :, pl.ds(8, 8), :], sem_c.at[0, 1]).start()
        pltpu.make_async_copy(xp_hbm.at[pl.ds(0, NP - 1), 1],
                              xc_s.at[0, pl.ds(1, NP - 1), :, pl.ds(0, 8), :], sem_c.at[0, 0]).start()
        xc_s[1, 0, :, pl.ds(0, 8), :] = jnp.zeros((NV, 8, 128), bf16)
        pltpu.make_async_copy(xc_s.at[1, 0, :, pl.ds(0, 8), :],
                              xc_s.at[0, 0, :, pl.ds(0, 8), :], sem_c.at[0, 0]).start()
        for c in cps:
            c.wait()

        for n in range(4):
            z_s[n] = 0
        acc_s[...] = jnp.zeros(acc_s.shape, f32)
        cl_s[...] = jnp.zeros(cl_s.shape, u32)
        od_s[...] = jnp.zeros(od_s.shape, f32)
        y_s[...] = jnp.zeros(y_s.shape, u32)
        gb_s[...] = jnp.zeros(gb_s.shape, f32)
        dwr_s[...] = jnp.zeros(dwr_s.shape, f32)
        gb_s[0:1, 0:E] = gam_ref[...].astype(f32).reshape(1, E)
        gb_s[1:2, 0:E] = bet_ref[...].astype(f32).reshape(1, E)
        w2s_s[...] = pltpu.bitcast(w2t_ref[...], u32)
        w1t_s[...] = pltpu.bitcast(jnp.transpose(w1_ref[...].astype(f32)).astype(bf16), u32)
        for i in range(3):
            for j in range(3):
                dwr_s[i * 3 + j:i * 3 + j + 1, 0:C] = dw_ref[i, j:j + 1, :].astype(f32)
        build_taps()
        r16 = jax.lax.broadcasted_iota(jnp.int32, (16, 128), 0)
        c16 = jax.lax.broadcasted_iota(jnp.int32, (16, 128), 1)
        kv = c16 // 16
        kb = c16 % 16
        k_row = 2 * (kv // 3) + kb // 8 - r16 // 8
        k_j = kv % 3
        for cg in range(NG):
            l1 = jnp.zeros((16, 128), f32)
            for i in range(3):
                for j in range(3):
                    w8 = wtap(i, j, cg)
                    hit = (kb % 8 == r16 % 8) & (k_row == i) & (k_j == j) & (kv < 6)
                    l1 = jnp.where(hit, jnp.concatenate([w8, w8], axis=0), l1)
            l1_s[cg] = pltpu.bitcast(l1.astype(bf16), u32)
        lr_s[NR - 1] = jnp.zeros(lr_s.shape[1:], u32)
        lr_s[NR - 2] = jnp.zeros(lr_s.shape[1:], u32)

    pl.run_scoped(
        setup,
        pltpu.VMEM((3, 3, C), bf16),
        pltpu.VMEM((C, E), bf16),
        pltpu.VMEM((C, E), bf16),
        pltpu.VMEM((E,), bf16),
        pltpu.VMEM((E,), bf16),
    )

    def a1(slot, q):
        for cg in range(NG):
            t = [xu[slot, q, cg * NT + k] for k in range(NT)]
            for k in range(NT):
                lo = (cg * NT + k) * 8
                if q == NP - 1:
                    cl_s[lo:lo + 8, :] = t[k]
                if q == NP - 2 and k >= NT - SH:
                    l2 = (NV + cg * SH + k - (NT - SH)) * 8
                    cl_s[l2:l2 + 8, :] = t[k]
                lsrc = t[k - 1] if k > 0 else zero_u
                rsrc = t[k + 1] if k < NT - 1 else zero_u
                lr_s[q % NR, 0, lo:lo + 8, :] = pltpu.roll(jnp.where(lane == 127, lsrc, t[k]), 1, 1)
                lr_s[q % NR, 1, lo:lo + 8, :] = pltpu.roll(jnp.where(lane == 0, rsrc, t[k]), 127, 1)

    def conv_pair_dot(slot, j, cg, k):
        n = cg * NT + k
        parts = []
        for q in (j, j + 1):
            m = n if q == -1 else NV + cg * SH + k - (NT - SH)
            c = xu[slot, q, n] if q >= 0 else cl_s[8 * m:8 * m + 8, :]
            parts += [lr_s[q % NR, 0, 8 * n:8 * n + 8, :], c, lr_s[q % NR, 1, 8 * n:8 * n + 8, :]]
        wt = pltpu.bitcast(jnp.concatenate(parts, axis=0), bf16)
        lhs = pltpu.bitcast(l1_s[cg, :, 0:96], bf16)
        return jnp.dot(lhs, wt, preferred_element_type=f32)

    def ln_unit(o, j, k, scale, link):
        ys = []
        for hh in range(2):
            yt = _layernorm_tile([o[q][8 * hh:8 * hh + 8] for q in range(NG)], C, scale, ys)
            y_b.at[j % NR, hh][:, k * 128:(k + 1) * 128] = yt
        if link:
            ys = [pltpu.bitcast(v, u32) for v in ys[LSTEP - 1::LSTEP]]
            dep = ys[0]
            for v in ys[1:]:
                dep = dep | v
            pend.append((link, dep))

    def dot_stream(slot, units, first_scale, defer):
        for u, (j, k) in enumerate(units):
            if k == 0 and j + 1 >= 0:
                a1(slot, j + 1)
            o = []
            for cg in range(NG):
                o.append(conv_pair_dot(slot, j, cg, k))
                if cg == NG - 1:
                    if u >= len(units) - defer:
                        od_s[u - (len(units) - defer)] = jnp.concatenate(o, axis=0)
                    else:
                        ln_unit(o, j, k, first_scale if j == -1 else ln_scale, 0)
                if cg % 4 == 3:
                    yield

    def deferred_ln():
        for d in range(ND):
            o = [od_s[d, 16 * cg:16 * cg + 16, :] for cg in range(NG)]
            ln_unit(o, -2, NT - SH - ND + d, ln_scale, HL)

    def c_stream(blk, pairs, gen, skip):
        n_gap = 0
        for jc in pairs:
            for n in range(2 * NCH):
                gelu_acc(mm1_raw(y_b[jc % NR, n // NCH], n % NCH, CH), n % NCH,
                         gindex(blk, 2 * jc + n // NCH))
                if n_gap >= skip:
                    next(gen, None)
                n_gap += 1

    carry_units = [(-2, k) for k in range(NT - SH, NT)]

    def p1_body(i, carry):
        slot = i & 1
        for c in c_copies(1, slot):
            c.wait()

        @pl.when(i + 1 < NB1)
        def _():
            for c in c_copies(i + 1, 1 - slot):
                c.start()

        @pl.when(i + 1 == NB1)
        def _():
            last_copy(1 - slot).start()

        deferred_ln()
        units = carry_units + [(j, k) for j in range(-1, NP - 1) for k in range(NT)]
        units = units[:NP * NT]
        gen = dot_stream(slot, units, jnp.where(i > 0, ln_scale, -1000.0), ND)
        c_stream(i, range(-3, NP - 3), gen, 0)
        assert next(gen, 'done') == 'done'
        return carry

    if not SKIP1:
        jax.lax.fori_loop(0, NB1, p1_body, 0)

    def xslot(s):
        return xc_s.at[s >> 1, pl.ds((s & 1) * (TH // 2), TH // 2)]

    def x_copy(blk, s):
        return pltpu.make_async_copy(x_hbm.at[pl.ds(blk * (TH // 2), TH // 2)], xslot(s), sem_x.at[s])

    def o_copy(blk, s):
        return pltpu.make_async_copy(xslot(s), o_hbm.at[pl.ds(blk * (TH // 2), TH // 2)], sem_o.at[s])

    dslot = NB1 % 2
    S0 = 2 * (1 - dslot)
    last_copy(dslot).wait()
    x_copy(0, S0).start()
    x_copy(1, S0 + 1).start()
    xc_s[dslot, 0, :, pl.ds(8, 8), :] = jnp.zeros((NV, 8, 128), bf16)
    if not SKIP1:
        deferred_ln()
        gen = dot_stream(dslot, carry_units + [(-1, k) for k in range(NT)], ln_scale, 0)
        c_stream(NB1, range(-3, 0), gen, 0)
        assert next(gen, 'done') == 'done'

    ssq = jnp.sum(jnp.transpose(acc_s[...]), axis=0, keepdims=True)
    gx = jnp.sqrt(ssq * (1.0 / (_GS * _GS)) + 1e-6)
    nx = gx / (jnp.sum(gx, axis=1, keepdims=True) * (1.0 / E) + 1e-6)
    sc = (gb_s[0:1, 0:E] * nx + 1.0) * (1.0 / _GS)
    w2 = pltpu.bitcast(w2s_s[...], bf16).astype(f32)
    w2s_s[...] = pltpu.bitcast((w2 * sc).astype(bf16), u32)
    b = jnp.sum(w2 * gb_s[1:2, 0:E], axis=1, keepdims=True)
    bias_s[...] = jnp.broadcast_to(b, (C, 128))
    build_taps()
    if DMAEND:
        x_copy(2, (S0 + 2) & 3).start()

    def pass2():

        def o_idx(n, k, cg):
            m = (n * NT + k) * NG + cg
            return (m // (2 * NV), (m // NV) % 2, pl.ds((m % NV) * 8, 8), slice(None))

        def p2_body(i, carry):
            s = (i + S0) & 3
            sa, sb = s >> 1, (s & 1) * (TH // 2)
            x_copy(0, s).wait()

            if not DMAEND:
                @pl.when(i >= 2)
                def _():
                    o_copy(0, (s + 2) & 3).wait()

                @pl.when(i + 2 < NB)
                def _():
                    x_copy(i + 2, (s + 2) & 3).start()

            def xrow(r, slab, tag=None):
                if tag is not None and OPQ == 2:
                    u = xu[sa, sb + z_s[tag] + r // 2, (r % 2) * NS + slab]
                else:
                    u = xu[sa, sb + r // 2, (r % 2) * NS + slab]
                if tag is not None and OPQ == 1:
                    u = u | jnp.full((8, 128), z_s[tag], jnp.int32).astype(u32)
                v = pltpu.bitcast(u, bf16).astype(f32)
                return [v[0:8], v[8:16]]

            def conv_piece(n, cgs):
                outs = []
                for cg in cgs:
                    rows_ = [xrow(r, 2 * cg, 1 + n) + xrow(r, 2 * cg + 1, 1 + n) for r in range(RC[n] - 1, RC[n] + 2)]
                    w = [[wtap(ii, j, cg) for j in range(3)] for ii in range(3)]
                    t = [[rows_[0][k] * w[0][j] + rows_[1][k] * w[1][j] + rows_[2][k] * w[2][j]
                          for k in range(NT)] for j in range(3)]
                    for k in range(NT):
                        lsrc = t[0][k - 1] if k > 0 else zero_f
                        rsrc = t[2][k + 1] if k < NT - 1 else zero_f
                        left = pltpu.roll(jnp.where(lane == 127, lsrc, t[0][k]), 1, 1)
                        right = pltpu.roll(jnp.where(lane == 0, rsrc, t[2][k]), 127, 1)
                        ov = pltpu.bitcast(t[1][k] + left + right, u32)
                        lr_s[o_idx(n, k, cg)] = ov
                        outs.append(ov)
                dep = outs[0]
                for v in outs[1:]:
                    dep = dep | v
                pend.append((LDIST, dep))

            done = [False] * len(RC)

            def pieces():
                for n in range(len(RC)):
                    for c0 in range(0, NG, PG):
                        conv_piece(n, range(c0, c0 + PG))
                        if c0 + PG == NG:
                            done[n] = True
                            for k in range(NT):
                                o = [pltpu.bitcast(lr_s[o_idx(n, k, cg)], f32) for cg in range(NG)]
                                ys = []
                                y_b.at[n // 2, n % 2][:, k * 128:(k + 1) * 128] = _layernorm_tile(
                                    o, C, ln_scale, ys)
                                if LNL:
                                    dep = pltpu.bitcast(ys[0], u32)
                                    for v in ys[1:]:
                                        dep = dep | pltpu.bitcast(v, u32)
                                    pend.append((LNL + (k if LNS else 0), dep))
                        yield

            def epilogue(r, p):
                assert all(done[n] for n in range(len(RC)) if abs(RC[n] - r) <= 1)
                for pp in range(NT // 2):
                    for cg in range(NG):
                        b8 = bias_s[cg * 8:cg * 8 + 8, :]
                        slab = 2 * cg + pp
                        xr = xrow(r, slab)
                        v = [xr[h] + (p[2 * pp + h][cg * 8:cg * 8 + 8] + b8) for h in range(2)]
                        xc_s[sa, sb + r // 2, (r % 2) * NS + slab] = jnp.concatenate(
                            v, axis=0).astype(bf16)

            def w2_lhs(c=None):
                u = w2s_s[...] if c is None else w2s_s[:, c * 128:(c + 1) * 128]
                return pltpu.bitcast(linked(u), bf16)

            pend.clear()
            res = list(RORD)
            gen = pieces()
            cur = []
            gch = {}
            part = {}
            late = []
            kpos = [0]
            for tok in P2.split(','):
                op = tok[0]
                if op == 'p':
                    next(gen)
                    for it in list(late):
                        if all(done[n] for n in range(len(RC)) if abs(RC[n] - it[0]) <= 1):
                            epilogue(*it)
                            late.remove(it)
                elif op in 'Rr':
                    r = res[0]
                    g = g_b.at[i * NRES + res_rows.index(r)]
                    if op == 'R':
                        pf = jnp.dot(w2_lhs(), g[...], preferred_element_type=f32)
                        cur = [pf[:, k * 128:(k + 1) * 128] for k in range(NT)]
                    else:
                        k = len(cur)
                        cur.append(jnp.dot(w2_lhs(), g[:, k * 128:(k + 1) * 128],
                                           preferred_element_type=f32))
                    if len(cur) == NT:
                        res.pop(0)
                        if all(done[n] for n in range(len(RC)) if abs(RC[n] - r) <= 1):
                            epilogue(r, cur)
                        else:
                            late.append((r, cur))
                        cur = []
                elif op == 'k':
                    r = res[0]
                    c = kpos[0]
                    g = g_b.at[i * NRES + res_rows.index(r)]
                    pf = jnp.dot(w2_lhs(c), g[c * 128:(c + 1) * 128, :], preferred_element_type=f32)
                    part['k'] = pf if c == 0 else part['k'] + pf
                    kpos[0] += 1
                    if c == E // 128 - 1:
                        kpos[0] = 0
                        res.pop(0)
                        it = (r, [part['k'][:, k * 128:(k + 1) * 128] for k in range(NT)])
                        if all(done[n] for n in range(len(RC)) if abs(RC[n] - r) <= 1):
                            epilogue(*it)
                        else:
                            late.append(it)
                elif op == 'x':
                    n, c = int(tok[1]), int(tok[2])
                    assert done[n]
                    gch[n, c] = _gelu2(mm1_raw(y_b[n // 2, n % 2], c, 128)).astype(bf16)
                elif op == 'X':
                    n = int(tok[1])
                    assert done[n]
                    gch[n] = _gelu2(mm1_raw(y_b[n // 2, n % 2], 0, E)).astype(bf16)
                elif op == 'A':
                    n = int(tok[1])
                    pf = jnp.dot(w2_lhs(), gch[n], preferred_element_type=f32)
                    epilogue(RC[n], [pf[:, k * 128:(k + 1) * 128] for k in range(NT)])
                elif op == 'a':
                    n, c = int(tok[1]), int(tok[2])
                    pf = jnp.dot(w2_lhs(c), gch[n, c], preferred_element_type=f32)
                    part[n] = pf if c == 0 else part[n] + pf
                    if c == E // 128 - 1:
                        epilogue(RC[n], [part[n][:, k * 128:(k + 1) * 128] for k in range(NT)])
            assert not res and not late and next(gen, 'done') == 'done'
            pend.clear()
            o_copy(i, s).start()
            if DMAEND:
                @pl.when(i >= 1)
                def _():
                    o_copy(0, (s + 3) & 3).wait()

                @pl.when(i + 3 < NB)
                def _():
                    x_copy(i + 3, (s + 3) & 3).start()
            return carry

        jax.lax.fori_loop(0, N2, p2_body, 0)
        if not DMAEND:
            o_copy(0, (N2 - 2 + S0) & 3).wait()
        o_copy(0, (N2 - 1 + S0) & 3).wait()
        if N2 < NB:
            x_copy(0, (N2 + S0) & 3).wait()
        if N2 + 1 < NB:
            x_copy(0, (N2 + 1 + S0) & 3).wait()
        if N2 + 2 < NB and DMAEND:
            x_copy(0, (N2 + 2 + S0) & 3).wait()

    pass2()


@jax.jit
def pallas_standalone__modern_conv_block_convnext_v2__vision_kernel(
    x: jax.Array,
    dw: jax.Array,
    w1: jax.Array,
    w2: jax.Array,
    grn_gamma: jax.Array,
    grn_beta: jax.Array,
):
    B, H, W, C = x.shape
    E = w1.shape[1]
    assert B == 1
    NB = H // TH
    NG = C // 8
    NT = W // 128
    NV = NG * NT
    x5 = jnp.transpose(x[0], (0, 2, 1)).reshape(H, NG, 8, NT, 128)
    x5 = jnp.transpose(x5, (0, 1, 3, 2, 4))
    xn = x5.reshape(H // 2, NV, 16, 128)
    xp = x5.reshape(H // 2, 2, NV, 8, 128)
    w2t = jnp.transpose(w2)

    kern = functools.partial(_kernel, H=H, C=C, E=E, W=W)
    hbm = pl.BlockSpec(memory_space=pl.ANY)
    out = pl.pallas_call(
        kern,
        in_specs=[hbm] * 7,
        out_specs=hbm,
        out_shape=jax.ShapeDtypeStruct((H // 2, NV, 16, 128), jnp.bfloat16),
        scratch_shapes=[
            pltpu.VMEM((NB * (TH - len(RC)) - GLESS, E // 2, W), u32),
            pltpu.VMEM((2, NP, NV, 16, 128), bf16),
            pltpu.VMEM((NR, 2, NV * 8, 128), u32),
            pltpu.VMEM((NR, 2, C // 2, W), u32),
            pltpu.VMEM(((NV + NG * 2) * 8, 128), u32),
            pltpu.VMEM((max(ND, 1), 2 * C, 128), f32),
            pltpu.VMEM((E, 128), f32),
            pltpu.VMEM((E // 2, C), u32),
            pltpu.VMEM((C // 2, E), u32),
            pltpu.VMEM((C, 128), f32),
            pltpu.VMEM((NG, 8, 128), u32),
            pltpu.VMEM((8, 512), f32),
            pltpu.VMEM((16, 128), f32),
            pltpu.SMEM((4,), jnp.int32),
            pltpu.SemaphoreType.DMA((2, 2)),
            pltpu.SemaphoreType.DMA((4,)),
            pltpu.SemaphoreType.DMA((4,)),
            pltpu.SemaphoreType.DMA((5,)),
        ],
        compiler_params=pltpu.CompilerParams(
            vmem_limit_bytes=128 * 1024 * 1024,
            disable_bounds_checks=True,
        ),
        name="convnext_block",
    )(xp, xn, dw, w1, w2t, grn_gamma, grn_beta)
    out = jnp.transpose(out.reshape(H, NG, NT, 8, 128), (0, 1, 3, 2, 4)).reshape(H, C, W)
    return jnp.transpose(out, (0, 2, 1))[None]
```

```python
import functools
import math

import jax
import jax.numpy as jnp
import jax.experimental.pallas as pl
import jax.experimental.pallas.tpu as pltpu

_K0 = math.sqrt(2.0 / math.pi)
_K1 = 0.044715 * _K0
_ALPHA = _K1 ** (1.0 / 3.0)
_KP = _K0 / _ALPHA
_GS = 2.0 * _ALPHA

f32 = jnp.float32
bf16 = jnp.bfloat16
u32 = jnp.uint32

NP = 8
NR = 4
LEAD = 3
CH = 64
TH = 8
RC = (1, 2, 3)
RES_ORDER = (5, 6, 7, 0, 4)
PG = 4
P2_ORDER = 'r,p,r,r,p,r,r,r,r,r,r,r,r,r,p,r,r,p,p,r,p,r,X0,p,p,r,r,p,r,X1,A0,r,X2,A1,A2'


def _tree_sum(vs):
    vs = list(vs)
    while len(vs) > 1:
        nxt = [vs[i] + vs[i + 1] for i in range(0, len(vs) - 1, 2)]
        if len(vs) % 2:
            nxt.append(vs[-1])
        vs = nxt
    return vs[0]


def _tree_or(vs):
    out = vs[0]
    for v in vs[1:]:
        out = out | v
    return out


def _sublane_allreduce(s):
    s = s + pltpu.roll(s, 4, 0)
    s = s + pltpu.roll(s, 2, 0)
    return s + pltpu.roll(s, 1, 0)


def _layernorm_tile(o):
    c = 8 * len(o)
    m = _sublane_allreduce(_tree_sum(o)) * (1.0 / c)
    d = [t - m for t in o]
    v = _sublane_allreduce(_tree_sum([t * t for t in d]))
    r = jnp.exp2(jnp.log(v + c * 1e-5) * (-0.5 * math.log2(math.e))
                 + math.log2(_ALPHA * math.sqrt(c)))
    return [t * r for t in d]


def _gelu2(h):
    return h * (1.0 + jnp.tanh(h * (h * h + _KP)))


def _kernel(xp_hbm, x_hbm, dw_hbm, w1_hbm, w2t_hbm, gam_hbm, bet_hbm,
            o_hbm,
            g_s, xc_s, lr_s, y_s, cl_s, od_s, acc_s, w1t_s, w2s_s, bias_s, l1_s, gb_s, dwr_s, z_s,
            sem_c, sem_x, sem_o, sem_p,
            *, H, C, E, W):
    NB1 = H // (2 * NP)
    NB2 = H // TH
    NG = C // 8
    NT = W // 128
    NS = NG * NT // 2
    NV = NG * NT
    NCH = E // CH
    res_rows = [r for r in range(TH) if r not in RC]
    NRES = len(res_rows)

    g_b = g_s.bitcast(bf16)
    y_b = y_s.bitcast(bf16)
    xu = xc_s.bitcast(u32)
    lane = jax.lax.broadcasted_iota(jnp.int32, (8, 128), 1)
    zero_u = jnp.zeros((8, 128), u32)
    zero_f = jnp.zeros((8, 128), f32)

    def tap_idx(t, lo, n):
        return (2 + t // 8, (t % 8) // 4, pl.ds((t % 4) * C + lo, n), slice(None))

    def build_taps():
        rows = jax.lax.broadcasted_iota(jnp.int32, (C, 128), 0)
        cols = jax.lax.broadcasted_iota(jnp.int32, (C, 128), 1)
        for t in range(9):
            col = jnp.sum(jnp.where(rows == cols, dwr_s[t:t + 1, :], 0.0), axis=1, keepdims=True)
            lr_s[tap_idx(t, 0, C)] = pltpu.bitcast(jnp.broadcast_to(col, (C, 128)), u32)

    def tap(i, j, cg):
        return pltpu.bitcast(lr_s[tap_idx(i * 3 + j, cg * 8, 8)], f32)

    pend = []

    def linked(u):
        due = [v for (n, v) in pend if n <= 1]
        pend[:] = [(n - 1, v) for (n, v) in pend if n > 1]
        if not due:
            return u
        dep = _tree_or(due) & jnp.full((8, 128), z_s[0], jnp.int32).astype(u32)
        if u.shape[1] <= 128:
            dep = dep[:, 0:u.shape[1]]
        else:
            dep = jnp.concatenate([dep, jnp.zeros((8, u.shape[1] - 128), u32)], axis=1)
        return jnp.concatenate([u[0:8] | dep, u[8:]], axis=0)

    def expand(y, lo, n):
        lhs = pltpu.bitcast(linked(w1t_s[lo // 2:(lo + n) // 2, :]), bf16)
        return _gelu2(jnp.dot(lhs, y, preferred_element_type=f32))

    NLAST = H // 2 - ((NB1 - 1) * NP + LEAD)

    def c_copies(blk, slot, n0=NP, n1=NP):
        q0 = blk * NP + LEAD
        return [
            pltpu.make_async_copy(xp_hbm.at[pl.ds(q0 - 1, n0), 1],
                                  xc_s.at[pl.ds(slot * NP, n0), :, pl.ds(0, 8), :], sem_c.at[slot, 0]),
            pltpu.make_async_copy(xp_hbm.at[pl.ds(q0, n1), 0],
                                  xc_s.at[pl.ds(slot * NP, n1), :, pl.ds(8, 8), :], sem_c.at[slot, 1]),
        ]

    def lead_copies():
        e0 = 2 * NP - LEAD
        return [
            pltpu.make_async_copy(xp_hbm.at[pl.ds(0, LEAD - 1), 1],
                                  xc_s.at[pl.ds(e0 + 1, LEAD - 1), :, pl.ds(0, 8), :], sem_c.at[1, 0]),
            pltpu.make_async_copy(xp_hbm.at[pl.ds(0, LEAD), 0],
                                  xc_s.at[pl.ds(e0, LEAD), :, pl.ds(8, 8), :], sem_c.at[1, 1]),
        ]

    S0 = 2 * (NB1 % 2)

    def x_copy(blk, s):
        return pltpu.make_async_copy(x_hbm.at[pl.ds(blk * (TH // 2), TH // 2)],
                                     xc_s.at[pl.ds(s * (TH // 2), TH // 2)], sem_x.at[s])

    def o_copy(blk, s):
        return pltpu.make_async_copy(xc_s.at[pl.ds(s * (TH // 2), TH // 2)],
                                     o_hbm.at[pl.ds(blk * (TH // 2), TH // 2)], sem_o.at[s])

    def setup(dw_ref, w1_ref, w2t_ref, gam_ref, bet_ref):
        bufs = (dw_ref, w1_ref, w2t_ref, gam_ref, bet_ref)
        cps = [pltpu.make_async_copy(src, dst, sem_p.at[n]) for n, (src, dst) in
               enumerate(zip((dw_hbm, w1_hbm, w2t_hbm, gam_hbm, bet_hbm), bufs))]
        for c in cps + lead_copies() + c_copies(0, 0):
            c.start()
        xc_s[2 * NP - LEAD, :, pl.ds(0, 8), :] = jnp.zeros((NV, 8, 128), bf16)
        for c in cps:
            c.wait()

        z_s[0] = 0
        acc_s[...] = jnp.zeros(acc_s.shape, f32)
        gb_s[...] = jnp.zeros(gb_s.shape, f32)
        dwr_s[...] = jnp.zeros(dwr_s.shape, f32)
        gb_s[0:1, 0:E] = gam_ref[...].astype(f32).reshape(1, E)
        gb_s[1:2, 0:E] = bet_ref[...].astype(f32).reshape(1, E)
        w2s_s[...] = pltpu.bitcast(w2t_ref[...], u32)
        w1t_s[...] = pltpu.bitcast(jnp.transpose(w1_ref[...].astype(f32)).astype(bf16), u32)
        for i in range(3):
            for j in range(3):
                dwr_s[i * 3 + j:i * 3 + j + 1, 0:C] = dw_ref[i, j:j + 1, :].astype(f32)
        build_taps()
        r16 = jax.lax.broadcasted_iota(jnp.int32, (16, 128), 0)
        c16 = jax.lax.broadcasted_iota(jnp.int32, (16, 128), 1)
        kv = c16 // 16
        kb = c16 % 16
        k_i = 2 * (kv // 3) + kb // 8 - r16 // 8
        k_j = kv % 3
        for cg in range(NG):
            l1 = jnp.zeros((16, 128), f32)
            for i in range(3):
                for j in range(3):
                    w8 = tap(i, j, cg)
                    hit = (kb % 8 == r16 % 8) & (k_i == i) & (k_j == j) & (kv < 6)
                    l1 = jnp.where(hit, jnp.concatenate([w8, w8], axis=0), l1)
            l1_s[cg] = pltpu.bitcast(l1.astype(bf16), u32)

    pl.run_scoped(
        setup,
        pltpu.VMEM((3, 3, C), bf16),
        pltpu.VMEM((C, E), bf16),
        pltpu.VMEM((C, E), bf16),
        pltpu.VMEM((E,), bf16),
        pltpu.VMEM((E,), bf16),
    )

    def shift_pair(slot, q):
        for cg in range(NG):
            t = [xu[slot * NP + q, cg * NT + k] for k in range(NT)]
            for k in range(NT):
                lo = (cg * NT + k) * 8
                if q == NP - 1:
                    cl_s[lo:lo + 8, :] = t[k]
                if q == NP - 2 and k == NT - 1:
                    cl_s[(NV + cg) * 8:(NV + cg) * 8 + 8, :] = t[k]
                lsrc = t[k - 1] if k > 0 else zero_u
                rsrc = t[k + 1] if k < NT - 1 else zero_u
                lr_s[q % NR, 0, lo:lo + 8, :] = pltpu.roll(jnp.where(lane == 127, lsrc, t[k]), 1, 1)
                lr_s[q % NR, 1, lo:lo + 8, :] = pltpu.roll(jnp.where(lane == 0, rsrc, t[k]), 127, 1)

    def conv_dot(slot, j, cg, k):
        n = cg * NT + k
        parts = []
        for q in (j, j + 1):
            m = n if q == -1 else NV + cg
            c = xu[slot * NP + q, n] if q >= 0 else cl_s[8 * m:8 * m + 8, :]
            parts += [lr_s[q % NR, 0, 8 * n:8 * n + 8, :], c, lr_s[q % NR, 1, 8 * n:8 * n + 8, :]]
        wt = pltpu.bitcast(jnp.concatenate(parts, axis=0), bf16)
        lhs = pltpu.bitcast(l1_s[cg, :, 0:96], bf16)
        return jnp.dot(lhs, wt, preferred_element_type=f32)

    def ln_unit(o, j, k):
        ys = []
        for hh in range(2):
            y = _layernorm_tile([o[cg][8 * hh:8 * hh + 8] for cg in range(NG)])
            y_b.at[j % NR, hh][:, k * 128:(k + 1) * 128] = jnp.concatenate(y, axis=0).astype(bf16)
            ys += y
        return ys

    def conv_stream(slot, units):
        for u, (j, k) in enumerate(units):
            if k == 0:
                shift_pair(slot, j + 1)
            o = []
            for cg in range(NG):
                o.append(conv_dot(slot, j, cg, k))
                if cg == NG - 1:
                    if u == len(units) - 1:
                        od_s[...] = jnp.concatenate(o, axis=0)
                    else:
                        ln_unit(o, j, k)
                if cg % 4 == 3:
                    yield

    for c in lead_copies():
        c.wait()
    shift_pair(1, NP - LEAD)
    for _ in conv_stream(1, [(j, k) for j in range(NP - LEAD, NP - 1) for k in range(NT)][:-1]):
        pass

    def p1_body(i, carry):
        slot = i & 1

        @pl.when(i + 1 < NB1)
        def _():
            for c in c_copies(0, slot):
                c.wait()

        @pl.when(i + 1 == NB1)
        def _():
            for c in c_copies(0, slot, NLAST + 1, NLAST):
                c.wait()

        @pl.when(i + 2 < NB1)
        def _():
            for c in c_copies(i + 1, 1 - slot):
                c.start()

        @pl.when(i + 2 == NB1)
        def _():
            for c in c_copies(NB1 - 1, (NB1 - 1) % 2, NLAST + 1, NLAST):
                c.start()
            xc_s[((NB1 - 1) % 2) * NP + NLAST, :, pl.ds(8, 8), :] = jnp.zeros((NV, 8, 128), bf16)

        @pl.when(i + 1 == NB1)
        def _():
            x_copy(0, S0).start()
            x_copy(1, S0 + 1).start()

        ys = ln_unit([od_s[16 * cg:16 * cg + 16, :] for cg in range(NG)], -2, NT - 2)
        pend.append((3, _tree_or([pltpu.bitcast(v, u32) for v in ys])))
        units = [(-2, NT - 1)] + [(j, k) for j in range(-1, NP - 1) for k in range(NT)][:-1]
        gen = conv_stream(slot, units)
        for r in range(2 * NP):
            res = r % TH in res_rows
            for c in range(NCH):
                g = expand(y_b[(r // 2 - LEAD) % NR, r % 2], c * CH, CH)
                g2 = g * g
                acc_s[c * CH:(c + 1) * CH, :] += _tree_sum(
                    [g2[:, k * 128:(k + 1) * 128] for k in range(NT)])
                if res:
                    gi = (i * (2 * NP // TH) + r // TH) * NRES + res_rows.index(r % TH)
                    g_b.at[gi][c * CH:(c + 1) * CH, :] = g.astype(bf16)
                next(gen)
        assert next(gen, 'done') == 'done' and not pend
        return carry

    jax.lax.fori_loop(0, NB1, p1_body, 0)
    x_copy(2, S0 + 2).start()

    ssq = jnp.sum(jnp.transpose(acc_s[...]), axis=0, keepdims=True)
    gx = jnp.sqrt(ssq * (1.0 / (_GS * _GS)) + 1e-6)
    nx = gx / (jnp.sum(gx, axis=1, keepdims=True) * (1.0 / E) + 1e-6)
    sc = (gb_s[0:1, 0:E] * nx + 1.0) * (1.0 / _GS)
    w2 = pltpu.bitcast(w2s_s[...], bf16).astype(f32)
    w2s_s[...] = pltpu.bitcast((w2 * sc).astype(bf16), u32)
    b = jnp.sum(w2 * gb_s[1:2, 0:E], axis=1, keepdims=True)
    bias_s[...] = jnp.broadcast_to(b, (C, 128))
    build_taps()

    def o_idx(n, k, cg):
        m = (n * NT + k) * NG + cg
        return (m // (2 * NV), (m // NV) % 2, pl.ds((m % NV) * 8, 8), slice(None))

    def p2_body(i, carry):
        s = (i + S0) & 3
        e0 = s * (TH // 2)
        x_copy(0, s).wait()

        def xrow(r, slab):
            v = pltpu.bitcast(xu[e0 + r // 2, (r % 2) * NS + slab], bf16).astype(f32)
            return [v[0:8], v[8:16]]

        done = [False] * len(RC)

        def pieces():
            for n in range(len(RC)):
                for c0 in range(0, NG, PG):
                    outs = []
                    for cg in range(c0, c0 + PG):
                        x3 = [xrow(r, 2 * cg) + xrow(r, 2 * cg + 1) for r in range(RC[n] - 1, RC[n] + 2)]
                        w = [[tap(ii, j, cg) for j in range(3)] for ii in range(3)]
                        t = [[x3[0][k] * w[0][j] + x3[1][k] * w[1][j] + x3[2][k] * w[2][j]
                              for k in range(NT)] for j in range(3)]
                        for k in range(NT):
                            lsrc = t[0][k - 1] if k > 0 else zero_f
                            rsrc = t[2][k + 1] if k < NT - 1 else zero_f
                            left = pltpu.roll(jnp.where(lane == 127, lsrc, t[0][k]), 1, 1)
                            right = pltpu.roll(jnp.where(lane == 0, rsrc, t[2][k]), 127, 1)
                            ov = pltpu.bitcast(t[1][k] + left + right, u32)
                            lr_s[o_idx(n, k, cg)] = ov
                            outs.append(ov)
                    pend.append((3, _tree_or(outs)))
                    if c0 + PG == NG:
                        done[n] = True
                        for k in range(NT):
                            y = _layernorm_tile(
                                [pltpu.bitcast(lr_s[o_idx(n, k, cg)], f32) for cg in range(NG)])
                            y_b.at[n // 2, n % 2][:, k * 128:(k + 1) * 128] = jnp.concatenate(
                                y, axis=0).astype(bf16)
                    yield

        def epilogue(r, p):
            assert all(done[n] for n in range(len(RC)) if abs(RC[n] - r) <= 1)
            for pp in range(NT // 2):
                for cg in range(NG):
                    b8 = bias_s[cg * 8:cg * 8 + 8, :]
                    slab = 2 * cg + pp
                    xr = xrow(r, slab)
                    v = [xr[h] + (p[2 * pp + h][cg * 8:cg * 8 + 8] + b8) for h in range(2)]
                    xc_s[e0 + r // 2, (r % 2) * NS + slab] = jnp.concatenate(v, axis=0).astype(bf16)

        def project(g):
            return jnp.dot(pltpu.bitcast(linked(w2s_s[...]), bf16), g, preferred_element_type=f32)

        rows = list(RES_ORDER)
        gen = pieces()
        cur = []
        act = {}
        for tok in P2_ORDER.split(','):
            if tok == 'p':
                next(gen)
            elif tok == 'r':
                k = len(cur)
                g = g_b.at[i * NRES + res_rows.index(rows[0])]
                cur.append(project(g[:, k * 128:(k + 1) * 128]))
                if len(cur) == NT:
                    epilogue(rows.pop(0), cur)
                    cur = []
            elif tok[0] == 'X':
                n = int(tok[1])
                assert done[n]
                act[n] = expand(y_b[n // 2, n % 2], 0, E).astype(bf16)
            else:
                n = int(tok[1])
                p = project(act[n])
                epilogue(RC[n], [p[:, k * 128:(k + 1) * 128] for k in range(NT)])
        assert not rows and next(gen, 'done') == 'done' and not pend

        o_copy(i, s).start()

        @pl.when(i >= 1)
        def _():
            o_copy(0, (s + 3) & 3).wait()

        @pl.when(i + 3 < NB2)
        def _():
            x_copy(i + 3, (s + 3) & 3).start()

        return carry

    jax.lax.fori_loop(0, NB2, p2_body, 0)
    o_copy(0, (NB2 - 1 + S0) & 3).wait()


@jax.jit
def pallas_standalone__modern_conv_block_convnext_v2__vision_kernel(
    x: jax.Array,
    dw: jax.Array,
    w1: jax.Array,
    w2: jax.Array,
    grn_gamma: jax.Array,
    grn_beta: jax.Array,
):
    B, H, W, C = x.shape
    E = w1.shape[1]
    assert B == 1
    NG = C // 8
    NT = W // 128
    NV = NG * NT
    x5 = jnp.transpose(x[0], (0, 2, 1)).reshape(H, NG, 8, NT, 128)
    x5 = jnp.transpose(x5, (0, 1, 3, 2, 4))
    xn = x5.reshape(H // 2, NV, 16, 128)
    xp = x5.reshape(H // 2, 2, NV, 8, 128)

    hbm = pl.BlockSpec(memory_space=pl.ANY)
    out = pl.pallas_call(
        functools.partial(_kernel, H=H, C=C, E=E, W=W),
        in_specs=[hbm] * 7,
        out_specs=hbm,
        out_shape=jax.ShapeDtypeStruct((H // 2, NV, 16, 128), jnp.bfloat16),
        scratch_shapes=[
            pltpu.VMEM((H // TH * (TH - len(RC)), E // 2, W), u32),
            pltpu.VMEM((2 * NP, NV, 16, 128), bf16),
            pltpu.VMEM((NR, 2, NV * 8, 128), u32),
            pltpu.VMEM((NR, 2, C // 2, W), u32),
            pltpu.VMEM(((NV + 2 * NG) * 8, 128), u32),
            pltpu.VMEM((2 * C, 128), f32),
            pltpu.VMEM((E, 128), f32),
            pltpu.VMEM((E // 2, C), u32),
            pltpu.VMEM((C // 2, E), u32),
            pltpu.VMEM((C, 128), f32),
            pltpu.VMEM((NG, 8, 128), u32),
            pltpu.VMEM((8, 512), f32),
            pltpu.VMEM((16, 128), f32),
            pltpu.SMEM((1,), jnp.int32),
            pltpu.SemaphoreType.DMA((2, 2)),
            pltpu.SemaphoreType.DMA((4,)),
            pltpu.SemaphoreType.DMA((4,)),
            pltpu.SemaphoreType.DMA((5,)),
        ],
        compiler_params=pltpu.CompilerParams(
            vmem_limit_bytes=128 * 1024 * 1024,
            disable_bounds_checks=True,
        ),
        name="convnext_block",
    )(xp, xn, dw, w1, jnp.transpose(w2), grn_gamma, grn_beta)
    out = jnp.transpose(out.reshape(H, NG, NT, 8, 128), (0, 1, 3, 2, 4)).reshape(H, C, W)
    return jnp.transpose(out, (0, 2, 1))[None]
```

```python
import functools
import math

import jax
import jax.numpy as jnp
import jax.experimental.pallas as pl
import jax.experimental.pallas.tpu as pltpu

_K0 = math.sqrt(2.0 / math.pi)
_K1 = 0.044715 * _K0
_ALPHA = _K1 ** (1.0 / 3.0)
_KP = _K0 / _ALPHA
_GS = 2.0 * _ALPHA

f32 = jnp.float32
bf16 = jnp.bfloat16
u32 = jnp.uint32

NP = 8
NR = 4
LEAD = 3
CH = 64
TH = 8
RC = (1, 2, 3)
RES_ORDER = (5, 6, 7, 0, 4)
PG = 4
P2_ORDER = 'r,p,r,r,r,r,r,r,p,r,r,r,p,r,r,r,r,p,p,r,p,r,X0,p,p,r,p,r,r,X1,A0,r,X2,A1,A2'


def _tree_sum(vs):
    vs = list(vs)
    while len(vs) > 1:
        nxt = [vs[i] + vs[i + 1] for i in range(0, len(vs) - 1, 2)]
        if len(vs) % 2:
            nxt.append(vs[-1])
        vs = nxt
    return vs[0]


def _tree_or(vs):
    out = vs[0]
    for v in vs[1:]:
        out = out | v
    return out


def _sublane_allreduce(s):
    s = s + pltpu.roll(s, 4, 0)
    s = s + pltpu.roll(s, 2, 0)
    return s + pltpu.roll(s, 1, 0)


def _layernorm_tile(o):
    c = 8 * len(o)
    m = _sublane_allreduce(_tree_sum(o)) * (1.0 / c)
    d = [t - m for t in o]
    v = _sublane_allreduce(_tree_sum([t * t for t in d]))
    r = jnp.exp2(jnp.log(v + c * 1e-5) * (-0.5 * math.log2(math.e))
                 + math.log2(_ALPHA * math.sqrt(c)))
    return [t * r for t in d]


def _gelu2(h):
    return h * (1.0 + jnp.tanh(h * (h * h + _KP)))


def _kernel(xp_hbm, x_hbm, dw_hbm, w1_hbm, w2t_hbm, gam_hbm, bet_hbm,
            o_hbm,
            g_s, xc_s, lr_s, y_s, cl_s, od_s, acc_s, w1t_s, w2s_s, bias_s, l1_s, gb_s, dwr_s, z_s,
            sem_c, sem_x, sem_o, sem_p,
            *, H, C, E, W):
    NB1 = H // (2 * NP)
    NB2 = H // TH
    NG = C // 8
    NT = W // 128
    NS = NG * NT // 2
    NV = NG * NT
    NCH = E // CH
    res_rows = [r for r in range(TH) if r not in RC]
    NRES = len(res_rows)

    g_b = g_s.bitcast(bf16)
    y_b = y_s.bitcast(bf16)
    xu = xc_s.bitcast(u32)
    lane = jax.lax.broadcasted_iota(jnp.int32, (8, 128), 1)
    zero_u = jnp.zeros((8, 128), u32)
    zero_f = jnp.zeros((8, 128), f32)

    def tap_idx(t, lo, n):
        return (2 + t // 8, (t % 8) // 4, pl.ds((t % 4) * C + lo, n), slice(None))

    def build_taps():
        rows = jax.lax.broadcasted_iota(jnp.int32, (C, 128), 0)
        cols = jax.lax.broadcasted_iota(jnp.int32, (C, 128), 1)
        ones = jnp.ones((128, 128), bf16)
        for t in range(9):
            diag = jnp.where(rows == cols, dwr_s[t:t + 1, :], 0.0).astype(bf16)
            lr_s[tap_idx(t, 0, C)] = pltpu.bitcast(
                jnp.dot(diag, ones, preferred_element_type=f32), u32)

    def tap(i, j, cg):
        return pltpu.bitcast(lr_s[tap_idx(i * 3 + j, cg * 8, 8)], f32)

    pend = []

    def linked(u):
        due = [v for (n, v) in pend if n <= 1]
        pend[:] = [(n - 1, v) for (n, v) in pend if n > 1]
        if not due:
            return u
        dep = _tree_or(due) & jnp.full((8, 128), z_s[0], jnp.int32).astype(u32)
        if u.shape[1] <= 128:
            dep = dep[:, 0:u.shape[1]]
        else:
            dep = jnp.concatenate([dep, jnp.zeros((8, u.shape[1] - 128), u32)], axis=1)
        return jnp.concatenate([u[0:8] | dep, u[8:]], axis=0)

    def expand(y, lo, n):
        lhs = pltpu.bitcast(linked(w1t_s[lo // 2:(lo + n) // 2, :]), bf16)
        return _gelu2(jnp.dot(lhs, y, preferred_element_type=f32))

    NLAST = H // 2 - ((NB1 - 1) * NP + LEAD)

    def c_copies(blk, slot, n0=NP, n1=NP):
        q0 = blk * NP + LEAD
        return [
            pltpu.make_async_copy(xp_hbm.at[pl.ds(q0 - 1, n0), 1],
                                  xc_s.at[pl.ds(slot * NP, n0), :, pl.ds(0, 8), :], sem_c.at[slot, 0]),
            pltpu.make_async_copy(xp_hbm.at[pl.ds(q0, n1), 0],
                                  xc_s.at[pl.ds(slot * NP, n1), :, pl.ds(8, 8), :], sem_c.at[slot, 1]),
        ]

    def lead_copies():
        e0 = 2 * NP - LEAD
        return [
            pltpu.make_async_copy(xp_hbm.at[pl.ds(0, LEAD - 1), 1],
                                  xc_s.at[pl.ds(e0 + 1, LEAD - 1), :, pl.ds(0, 8), :], sem_c.at[1, 0]),
            pltpu.make_async_copy(xp_hbm.at[pl.ds(0, LEAD), 0],
                                  xc_s.at[pl.ds(e0, LEAD), :, pl.ds(8, 8), :], sem_c.at[1, 1]),
        ]

    S0 = 2 * (NB1 % 2)

    def x_copy(blk, s):
        return pltpu.make_async_copy(x_hbm.at[pl.ds(blk * (TH // 2), TH // 2)],
                                     xc_s.at[pl.ds(s * (TH // 2), TH // 2)], sem_x.at[s])

    def o_copy(blk, s):
        return pltpu.make_async_copy(xc_s.at[pl.ds(s * (TH // 2), TH // 2)],
                                     o_hbm.at[pl.ds(blk * (TH // 2), TH // 2)], sem_o.at[s])

    def setup(dw_ref, w1_ref, w2t_ref, gam_ref, bet_ref):
        bufs = (dw_ref, w1_ref, w2t_ref, gam_ref, bet_ref)
        cps = [pltpu.make_async_copy(src, dst, sem_p.at[n]) for n, (src, dst) in
               enumerate(zip((dw_hbm, w1_hbm, w2t_hbm, gam_hbm, bet_hbm), bufs))]
        for c in cps + lead_copies() + c_copies(0, 0):
            c.start()
        xc_s[2 * NP - LEAD, :, pl.ds(0, 8), :] = jnp.zeros((NV, 8, 128), bf16)
        for c in cps:
            c.wait()

        z_s[0] = 0
        acc_s[...] = jnp.zeros(acc_s.shape, f32)
        gb_s[...] = jnp.zeros(gb_s.shape, f32)
        dwr_s[...] = jnp.zeros(dwr_s.shape, f32)
        gb_s[0:1, 0:E] = gam_ref[...].astype(f32).reshape(1, E)
        beta = bet_ref[...].astype(f32).reshape(1, E)
        b = jnp.sum(w2t_ref[...].astype(f32) * beta, axis=1, keepdims=True)
        bias_s[...] = jnp.broadcast_to(b, (C, 128))
        w2s_s[...] = pltpu.bitcast(w2t_ref[...], u32)
        w1t_s[...] = pltpu.bitcast(jnp.transpose(w1_ref[...].astype(f32)).astype(bf16), u32)
        for i in range(3):
            for j in range(3):
                dwr_s[i * 3 + j:i * 3 + j + 1, 0:C] = dw_ref[i, j:j + 1, :].astype(f32)
        build_taps()
        r16 = jax.lax.broadcasted_iota(jnp.int32, (16, 128), 0)
        c16 = jax.lax.broadcasted_iota(jnp.int32, (16, 128), 1)
        kv = c16 // 16
        kb = c16 % 16
        k_i = 2 * (kv // 3) + kb // 8 - r16 // 8
        k_j = kv % 3
        for cg in range(NG):
            l1 = jnp.zeros((16, 128), f32)
            for i in range(3):
                for j in range(3):
                    w8 = tap(i, j, cg)
                    hit = (kb % 8 == r16 % 8) & (k_i == i) & (k_j == j) & (kv < 6)
                    l1 = jnp.where(hit, jnp.concatenate([w8, w8], axis=0), l1)
            l1_s[cg] = pltpu.bitcast(l1.astype(bf16), u32)

    pl.run_scoped(
        setup,
        pltpu.VMEM((3, 3, C), bf16),
        pltpu.VMEM((C, E), bf16),
        pltpu.VMEM((C, E), bf16),
        pltpu.VMEM((E,), bf16),
        pltpu.VMEM((E,), bf16),
    )

    def shift_pair(slot, q):
        for cg in range(NG):
            t = [xu[slot * NP + q, cg * NT + k] for k in range(NT)]
            for k in range(NT):
                lo = (cg * NT + k) * 8
                if q == NP - 1:
                    cl_s[lo:lo + 8, :] = t[k]
                if q == NP - 2 and k == NT - 1:
                    cl_s[(NV + cg) * 8:(NV + cg) * 8 + 8, :] = t[k]
                lsrc = t[k - 1] if k > 0 else zero_u
                rsrc = t[k + 1] if k < NT - 1 else zero_u
                lr_s[q % NR, 0, lo:lo + 8, :] = pltpu.roll(jnp.where(lane == 127, lsrc, t[k]), 1, 1)
                lr_s[q % NR, 1, lo:lo + 8, :] = pltpu.roll(jnp.where(lane == 0, rsrc, t[k]), 127, 1)

    def conv_dot(slot, j, cg, k):
        n = cg * NT + k
        parts = []
        for q in (j, j + 1):
            m = n if q == -1 else NV + cg
            c = xu[slot * NP + q, n] if q >= 0 else cl_s[8 * m:8 * m + 8, :]
            parts += [lr_s[q % NR, 0, 8 * n:8 * n + 8, :], c, lr_s[q % NR, 1, 8 * n:8 * n + 8, :]]
        wt = pltpu.bitcast(jnp.concatenate(parts, axis=0), bf16)
        lhs = pltpu.bitcast(l1_s[cg, :, 0:96], bf16)
        return jnp.dot(lhs, wt, preferred_element_type=f32)

    def ln_unit(o, j, k):
        ys = []
        for hh in range(2):
            y = _layernorm_tile([o[cg][8 * hh:8 * hh + 8] for cg in range(NG)])
            y_b.at[j % NR, hh][:, k * 128:(k + 1) * 128] = jnp.concatenate(y, axis=0).astype(bf16)
            ys += y
        return ys

    def conv_stream(slot, units):
        for u, (j, k) in enumerate(units):
            if k == 0:
                shift_pair(slot, j + 1)
            o = []
            for cg in range(NG):
                o.append(conv_dot(slot, j, cg, k))
                if cg == NG - 1:
                    if u == len(units) - 1:
                        od_s[...] = jnp.concatenate(o, axis=0)
                    else:
                        ln_unit(o, j, k)
                if cg % 4 == 3:
                    yield

    for c in lead_copies():
        c.wait()
    shift_pair(1, NP - LEAD)
    for _ in conv_stream(1, [(j, k) for j in range(NP - LEAD, NP - 1) for k in range(NT)][:-1]):
        pass

    def p1_body(i, carry):
        slot = i & 1

        @pl.when(i + 1 < NB1)
        def _():
            for c in c_copies(0, slot):
                c.wait()

        @pl.when(i + 1 == NB1)
        def _():
            for c in c_copies(0, slot, NLAST + 1, NLAST):
                c.wait()

        @pl.when(i + 2 < NB1)
        def _():
            for c in c_copies(i + 1, 1 - slot):
                c.start()

        @pl.when(i + 2 == NB1)
        def _():
            for c in c_copies(NB1 - 1, (NB1 - 1) % 2, NLAST + 1, NLAST):
                c.start()
            xc_s[((NB1 - 1) % 2) * NP + NLAST, :, pl.ds(8, 8), :] = jnp.zeros((NV, 8, 128), bf16)

        @pl.when(i + 1 == NB1)
        def _():
            x_copy(0, S0).start()
            x_copy(1, S0 + 1).start()

        ys = ln_unit([od_s[16 * cg:16 * cg + 16, :] for cg in range(NG)], -2, NT - 2)
        pend.append((3, _tree_or([pltpu.bitcast(v, u32) for v in ys])))
        units = [(-2, NT - 1)] + [(j, k) for j in range(-1, NP - 1) for k in range(NT)][:-1]
        gen = conv_stream(slot, units)
        for r in range(2 * NP):
            res = r % TH in res_rows
            for c in range(NCH):
                g = expand(y_b[(r // 2 - LEAD) % NR, r % 2], c * CH, CH)
                if res:
                    gi = (i * (2 * NP // TH) + r // TH) * NRES + res_rows.index(r % TH)
                    g_b.at[gi][c * CH:(c + 1) * CH, :] = g.astype(bf16)
                g2 = g * g
                acc_s[c * CH:(c + 1) * CH, :] += _tree_sum(
                    [g2[:, k * 128:(k + 1) * 128] for k in range(NT)])
                next(gen)
        assert next(gen, 'done') == 'done' and not pend
        return carry

    jax.lax.fori_loop(0, NB1, p1_body, 0)
    x_copy(2, (S0 + 2) & 3).start()

    ssq = jnp.sum(jnp.transpose(acc_s[...]), axis=0, keepdims=True)
    gx = jnp.sqrt(ssq * (1.0 / (_GS * _GS)) + 1e-6)
    nx = gx / (jnp.sum(gx, axis=1, keepdims=True) * (1.0 / E) + 1e-6)
    sc = (gb_s[0:1, 0:E] * nx + 1.0) * (1.0 / _GS)
    w2 = pltpu.bitcast(w2s_s[...], bf16).astype(f32)
    w2s_s[...] = pltpu.bitcast((w2 * sc).astype(bf16), u32)
    build_taps()

    def o_idx(n, k, cg):
        m = (n * NT + k) * NG + cg
        return (m // (2 * NV), (m // NV) % 2, pl.ds((m % NV) * 8, 8), slice(None))

    def p2_body(i, carry):
        s = (i + S0) & 3
        e0 = s * (TH // 2)
        x_copy(0, s).wait()

        def xrow(r, slab):
            v = pltpu.bitcast(xu[e0 + r // 2, (r % 2) * NS + slab], bf16).astype(f32)
            return [v[0:8], v[8:16]]

        done = [False] * len(RC)

        def pieces():
            for n in range(len(RC)):
                for c0 in range(0, NG, PG):
                    outs = []
                    for cg in range(c0, c0 + PG):
                        x3 = [xrow(r, 2 * cg) + xrow(r, 2 * cg + 1) for r in range(RC[n] - 1, RC[n] + 2)]
                        w = [[tap(ii, j, cg) for j in range(3)] for ii in range(3)]
                        t = [[x3[0][k] * w[0][j] + x3[1][k] * w[1][j] + x3[2][k] * w[2][j]
                              for k in range(NT)] for j in range(3)]
                        for k in range(NT):
                            lsrc = t[0][k - 1] if k > 0 else zero_f
                            rsrc = t[2][k + 1] if k < NT - 1 else zero_f
                            left = pltpu.roll(jnp.where(lane == 127, lsrc, t[0][k]), 1, 1)
                            right = pltpu.roll(jnp.where(lane == 0, rsrc, t[2][k]), 127, 1)
                            ov = pltpu.bitcast(t[1][k] + left + right, u32)
                            lr_s[o_idx(n, k, cg)] = ov
                            outs.append(ov)
                    pend.append((3, _tree_or(outs)))
                    if c0 + PG == NG:
                        done[n] = True
                        for k in range(NT):
                            y = _layernorm_tile(
                                [pltpu.bitcast(lr_s[o_idx(n, k, cg)], f32) for cg in range(NG)])
                            y_b.at[n // 2, n % 2][:, k * 128:(k + 1) * 128] = jnp.concatenate(
                                y, axis=0).astype(bf16)
                    yield

        def epilogue(r, p):
            assert all(done[n] for n in range(len(RC)) if abs(RC[n] - r) <= 1)
            for pp in range(NT // 2):
                for cg in range(NG):
                    b8 = bias_s[cg * 8:cg * 8 + 8, :]
                    slab = 2 * cg + pp
                    xr = xrow(r, slab)
                    v = [xr[h] + (p[2 * pp + h][cg * 8:cg * 8 + 8] + b8) for h in range(2)]
                    xc_s[e0 + r // 2, (r % 2) * NS + slab] = jnp.concatenate(v, axis=0).astype(bf16)

        def project(g):
            return jnp.dot(pltpu.bitcast(linked(w2s_s[...]), bf16), g, preferred_element_type=f32)

        rows = list(RES_ORDER)
        gen = pieces()
        cur = []
        act = {}
        for tok in P2_ORDER.split(','):
            if tok == 'p':
                next(gen)
            elif tok == 'r':
                k = len(cur)
                g = g_b.at[i * NRES + res_rows.index(rows[0])]
                cur.append(project(g[:, k * 128:(k + 1) * 128]))
                if len(cur) == NT:
                    epilogue(rows.pop(0), cur)
                    cur = []
            elif tok[0] == 'X':
                n = int(tok[1])
                assert done[n]
                act[n] = expand(y_b[n // 2, n % 2], 0, E).astype(bf16)
            else:
                n = int(tok[1])
                p = project(act[n])
                epilogue(RC[n], [p[:, k * 128:(k + 1) * 128] for k in range(NT)])
        assert not rows and next(gen, 'done') == 'done' and not pend

        o_copy(i, s).start()

        @pl.when(i >= 1)
        def _():
            o_copy(0, (s + 3) & 3).wait()

        @pl.when(i + 3 < NB2)
        def _():
            x_copy(i + 3, (s + 3) & 3).start()

        return carry

    jax.lax.fori_loop(0, NB2, p2_body, 0)
    o_copy(0, (NB2 - 1 + S0) & 3).wait()


@jax.jit
def pallas_standalone__modern_conv_block_convnext_v2__vision_kernel(
    x: jax.Array,
    dw: jax.Array,
    w1: jax.Array,
    w2: jax.Array,
    grn_gamma: jax.Array,
    grn_beta: jax.Array,
):
    B, H, W, C = x.shape
    E = w1.shape[1]
    assert B == 1
    NG = C // 8
    NT = W // 128
    NV = NG * NT
    x5 = jnp.transpose(x[0], (0, 2, 1)).reshape(H, NG, 8, NT, 128)
    x5 = jnp.transpose(x5, (0, 1, 3, 2, 4))
    xn = x5.reshape(H // 2, NV, 16, 128)
    xp = x5.reshape(H // 2, 2, NV, 8, 128)

    hbm = pl.BlockSpec(memory_space=pl.ANY)
    out = pl.pallas_call(
        functools.partial(_kernel, H=H, C=C, E=E, W=W),
        in_specs=[hbm] * 7,
        out_specs=hbm,
        out_shape=jax.ShapeDtypeStruct((H // 2, NV, 16, 128), jnp.bfloat16),
        scratch_shapes=[
            pltpu.VMEM((H // TH * (TH - len(RC)), E // 2, W), u32),
            pltpu.VMEM((2 * NP, NV, 16, 128), bf16),
            pltpu.VMEM((NR, 2, NV * 8, 128), u32),
            pltpu.VMEM((NR, 2, C // 2, W), u32),
            pltpu.VMEM(((NV + 2 * NG) * 8, 128), u32),
            pltpu.VMEM((2 * C, 128), f32),
            pltpu.VMEM((E, 128), f32),
            pltpu.VMEM((E // 2, C), u32),
            pltpu.VMEM((C // 2, E), u32),
            pltpu.VMEM((C, 128), f32),
            pltpu.VMEM((NG, 8, 128), u32),
            pltpu.VMEM((8, 512), f32),
            pltpu.VMEM((16, 128), f32),
            pltpu.SMEM((1,), jnp.int32),
            pltpu.SemaphoreType.DMA((2, 2)),
            pltpu.SemaphoreType.DMA((4,)),
            pltpu.SemaphoreType.DMA((4,)),
            pltpu.SemaphoreType.DMA((5,)),
        ],
        compiler_params=pltpu.CompilerParams(
            vmem_limit_bytes=128 * 1024 * 1024,
            disable_bounds_checks=True,
        ),
        name="convnext_block",
    )(xp, xn, dw, w1, jnp.transpose(w2), grn_gamma, grn_beta)
    out = jnp.transpose(out.reshape(H, NG, NT, 8, 128), (0, 1, 3, 2, 4)).reshape(H, C, W)
    return jnp.transpose(out, (0, 2, 1))[None]
```
